```python
import os as _os
_os.environ.setdefault("JAX_PLATFORMS", "cpu")
import jax
import jax.numpy as jnp

def _softmax(x, axis=-1):
    return jax.nn.softmax(x, axis=axis)
def _gelu(x):
    return jax.nn.gelu(x, approximate=True)
def _silu(x):
    return jax.nn.silu(x)
def _sigmoid(x):
    return jax.nn.sigmoid(x)
def _layernorm(x, axis=-1, eps=1e-5):
    m = jnp.mean(x, axis=axis, keepdims=True)
    v = jnp.var(x, axis=axis, keepdims=True)
    return (x - m) / jnp.sqrt(v + eps)
def _scatter_add(tgt, idx, src, axis=0):
    return tgt.at[idx].add(src)
def _segment_sum(src, seg, n):
    return jax.ops.segment_sum(src, seg, n)
class _Rng:
    def __init__(self, key):
        self._k = key
    def _next(self):
        self._k, sub = jax.random.split(self._k)
        return sub
    def normal(self, shape):
        return jax.random.normal(self._next(), shape, dtype=jnp.bfloat16)
    def randint(self, lo, hi, shape):
        return jax.random.randint(self._next(), shape, lo, hi, dtype=jnp.int32)
    def uniform(self, shape, lo=0.0, hi=1.0):
        return jax.random.uniform(self._next(), shape, jnp.bfloat16, lo, hi)
    def permutation(self, n):
        return jax.random.permutation(self._next(), n)


kernel_name = 'gated_mix__linear_attn_block__mixer_token_mlp__prompt'

def setup_inputs():
    _rng = _Rng(jax.random.key(int.from_bytes(__import__("os").urandom(4), "little")))
    _w = (lambda a: (lambda t: t.astype(jnp.bfloat16) if jnp.issubdtype(t.dtype, jnp.floating) else t)(jnp.asarray(a)))
    def _A_setup():
        B, S, D = 1, 2048, 512
        return {
            "x": _w((lambda *s: _rng.normal(s) * 0.05)(B, S, D)),
            "wqkv": _w((lambda *s: _rng.normal(s) * 0.8)(D, 3 * D)),
            "wo": _w((lambda *s: _rng.normal(s) * 0.05)(D, D)),
        }
    _A_in = _A_setup()

    def _B_setup():
        B, S, D, F = 1, 2048, 512, 1792
        return {
            "x": _w((lambda *s: _rng.normal(s) * 0.05)(B, S, D)),
            "w1": _w((lambda *s: _rng.normal(s) * 0.1)(S, F) * (S ** -0.5)),
            "b1": _w((lambda *s: _rng.normal(s) * 0.1)(F) * 0.02),
            "w2": _w((lambda *s: _rng.normal(s) * 0.1)(F, S) * (F ** -0.5)),
            "b2": _w((lambda *s: _rng.normal(s) * 0.1)(S) * 0.02),
        }
    _B_in = _B_setup()

    return {
        "A_x": _A_in["x"],
        "A_wqkv": _A_in["wqkv"],
        "A_wo": _A_in["wo"],
        "B_x": _B_in["x"],
        "B_w1": _B_in["w1"],
        "B_b1": _B_in["b1"],
        "B_w2": _B_in["w2"],
        "B_b2": _B_in["b2"],
        "gate_w": _w((lambda *s: _rng.normal(s) * 0.05)(512) * 16.0),
    }

def reference(A_x, A_wqkv, A_wo, B_x, B_w1, B_b1, B_w2, B_b2, gate_w):
    def _A_ref(x, wqkv, wo):
        B, S, D = x.shape
        H = 32; Dh = D // H
        qkv = (lambda x, *d: x.transpose(*d))((x @ wqkv).reshape(B, S, 3, H, Dh), 2, 0, 3, 1, 4)
        q, k, v = qkv[0], qkv[1], qkv[2]
        phi = lambda t: jnp.where(t > 0, t + 1, jnp.exp(t)) + 1e-6
        pq, pk = phi(q), phi(k)
        kv = jnp.einsum("bhsd,bhse->bhde", pk, v)
        z = jnp.einsum("bhsd->bhd", pk)
        num = jnp.einsum("bhqd,bhde->bhqe", pq, kv)
        den = jnp.einsum("bhqd,bhd->bhq", pq, z)[..., None] + 1e-6
        o = num / den
        return (lambda x, *d: x.transpose(*d))(o, 0, 2, 1, 3).reshape(B, S, D) @ wo

    def _B_ref(x, w1, b1, w2, b2):
        B, S, D = x.shape
        h = _layernorm(x, axis=-1)
        u = jnp.einsum("bsd,sf->bdf", h, w1) + b1
        u = _gelu(u)
        y = jnp.einsum("bdf,fs->bds", u, w2) + b2
        return (lambda x, *d: x.transpose(*d))(y, 0, 2, 1)

    x = A_x
    g = _sigmoid((x * gate_w).sum(-1, keepdims=True))
    a = _A_ref(x, A_wqkv, A_wo)
    b = _B_ref(x, B_w1, B_b1, B_w2, B_b2)
    return g * a + (1 - g) * b
```

```python
import jax
import jax.numpy as jnp
import jax.experimental.pallas as pl
import jax.experimental.pallas.tpu as pltpu

S, D, F = 2048, 512, 1792
H = 32
DH = D // H
G = 128
NG = D // G
TF = 256
TS = 256
NF = F // TF
NS = S // TS


def _phi(t):
    return jnp.where(t > 0, t + 1.0, jnp.exp(t)) + 1e-6


def _kernel(x_ref, wqkv_ref, wo_ref, w1_ref, b1_ref, w2_ref, b2_ref, gw_ref,
            o_ref, hT_ref, u_ref, kv_ref, w_ref):
    step = pl.program_id(0)

    @pl.when(step == 0)
    def _stats():
        z_row = jnp.zeros((1, D), jnp.float32)
        for g in range(NG):
            kv_ref[g] = jnp.zeros((G, G), jnp.float32)
        for c in range(NS):
            xb = x_ref[c * TS:(c + 1) * TS, :]
            xc = xb.astype(jnp.float32)
            m = jnp.mean(xc, axis=-1, keepdims=True)
            xm = xc - m
            var = jnp.mean(xm * xm, axis=-1, keepdims=True)
            h = xm / jnp.sqrt(var + 1e-5)
            hT_ref[:, c * TS:(c + 1) * TS] = h.T.astype(jnp.bfloat16)
            kv = jnp.dot(xb, wqkv_ref[:, D:3 * D],
                         preferred_element_type=jnp.float32)
            pk = _phi(kv[:, :D])
            z_row = z_row + jnp.sum(pk, axis=0, keepdims=True)
            pkT = pk.T.astype(jnp.bfloat16)
            vb = kv[:, D:].astype(jnp.bfloat16)
            for g in range(NG):
                kv_ref[g] += jnp.dot(pkT[g * G:(g + 1) * G, :],
                                     vb[:, g * G:(g + 1) * G],
                                     preferred_element_type=jnp.float32)
        ri = jax.lax.broadcasted_iota(jnp.int32, (G, G), 0) // DH
        ci = jax.lax.broadcasted_iota(jnp.int32, (G, G), 1) // DH
        mask = ri == ci
        for g in range(NG):
            zb = jnp.broadcast_to(z_row[:, g * G:(g + 1) * G], (G, G)).T
            w_ref[g * G:(g + 1) * G, 0:G] = jnp.where(
                mask, kv_ref[g], 0.0).astype(jnp.bfloat16)
            w_ref[g * G:(g + 1) * G, G:2 * G] = jnp.where(
                mask, zb, 0.0).astype(jnp.bfloat16)

    @pl.when(step < NF)
    def _mixer1():
        u = jnp.dot(hT_ref[...], w1_ref[...],
                    preferred_element_type=jnp.float32)
        u = u + b1_ref[...].astype(jnp.float32)
        off = pl.multiple_of(step * TF, TF)
        u_ref[:, pl.ds(off, TF)] = jax.nn.gelu(u, approximate=True).astype(
            jnp.bfloat16)

    @pl.when(step >= NF)
    def _out():
        c = step - NF
        off = pl.multiple_of(c * TS, TS)
        xb = x_ref[pl.ds(off, TS), :]
        xc = xb.astype(jnp.float32)
        gl = jnp.sum(xc * gw_ref[...].astype(jnp.float32), axis=-1,
                     keepdims=True)
        gate = jax.nn.sigmoid(gl)
        q = jnp.dot(xb, wqkv_ref[:, 0:D],
                    preferred_element_type=jnp.float32)
        pq = _phi(q).astype(jnp.bfloat16)
        os = []
        for g in range(NG):
            nd = jnp.dot(pq[:, g * G:(g + 1) * G], w_ref[g * G:(g + 1) * G, :],
                         preferred_element_type=jnp.float32)
            os.append(nd[:, :G] / (nd[:, G:] + 1e-6))
        o = jnp.concatenate(os, axis=-1).astype(jnp.bfloat16)
        a = jnp.dot(o, wo_ref[...], preferred_element_type=jnp.float32)
        y = jnp.dot(u_ref[...], w2_ref[...],
                    preferred_element_type=jnp.float32)
        y = y + b2_ref[...].astype(jnp.float32)
        b = y.T
        o_ref[...] = (gate * a + (1.0 - gate) * b).astype(o_ref.dtype)


@jax.jit
def pallas_gated_mix__linear_attn_block__mixer_token_mlp__prompt_kernel(
    A_x: jax.Array,
    A_wqkv: jax.Array,
    A_wo: jax.Array,
    B_x: jax.Array,
    B_w1: jax.Array,
    B_b1: jax.Array,
    B_w2: jax.Array,
    B_b2: jax.Array,
    gate_w: jax.Array,
):
    x = A_x.reshape(S, D)
    b1 = B_b1.reshape(1, F)
    b2 = B_b2.reshape(1, S)
    gw = gate_w.reshape(1, D)

    out = pl.pallas_call(
        _kernel,
        grid=(NF + NS,),
        in_specs=[
            pl.BlockSpec((S, D), lambda i: (0, 0)),
            pl.BlockSpec((D, 3 * D), lambda i: (0, 0)),
            pl.BlockSpec((D, D), lambda i: (0, 0)),
            pl.BlockSpec((S, TF), lambda i: (0, jnp.minimum(i, NF - 1))),
            pl.BlockSpec((1, TF), lambda i: (0, jnp.minimum(i, NF - 1))),
            pl.BlockSpec((F, TS), lambda i: (0, jnp.maximum(i - NF, 0))),
            pl.BlockSpec((1, TS), lambda i: (0, jnp.maximum(i - NF, 0))),
            pl.BlockSpec((1, D), lambda i: (0, 0)),
        ],
        out_specs=pl.BlockSpec((TS, D), lambda i: (jnp.maximum(i - NF, 0), 0)),
        out_shape=jax.ShapeDtypeStruct((S, D), A_x.dtype),
        scratch_shapes=[
            pltpu.VMEM((D, S), jnp.bfloat16),
            pltpu.VMEM((D, F), jnp.bfloat16),
            pltpu.VMEM((NG, G, G), jnp.float32),
            pltpu.VMEM((D, 2 * G), jnp.bfloat16),
        ],
        compiler_params=pltpu.CompilerParams(
            dimension_semantics=("arbitrary",),
            vmem_limit_bytes=64 * 1024 * 1024,
        ),
    )(x, A_wqkv, A_wo, B_w1, b1, B_w2, b2, gw)
    return out.reshape(1, S, D)
```

```python
import jax
import jax.numpy as jnp
import jax.experimental.pallas as pl
import jax.experimental.pallas.tpu as pltpu

S, D, F = 2048, 512, 1792
H = 32
DH = D // H
G = 128
NG = D // G
TF = 256
TS = 256
NF = F // TF
NS = S // TS

SEM_X = 0
SEM_W1 = SEM_X + NS
SEM_W2 = SEM_W1 + NF
SEM_WKV = SEM_W2 + NS
SEM_WQ = SEM_WKV + 1
SEM_WO = SEM_WQ + 1
NSEM = SEM_WO + 1


def _phi(t):
    return jnp.where(t > 0, t + 1.0, jnp.exp(t)) + 1e-6


def _kernel(x_hbm, wqkv_hbm, wo_hbm, w1_hbm, w2_hbm, b1_ref, b2_ref, gw_ref,
            o_ref,
            x_v, wkv_v, wq_v, wo_v, w1_v, w2_v, hT_ref, u_ref, kv_ref, z_ref,
            w_ref, sem):
    step = pl.program_id(0)

    def x_copy(c):
        off = pl.multiple_of(c * TS, TS)
        return pltpu.make_async_copy(x_hbm.at[pl.ds(off, TS), :],
                                     x_v.at[pl.ds(off, TS), :],
                                     sem.at[SEM_X + c])

    def w1_copy(j):
        off = pl.multiple_of(j * TF, TF)
        return pltpu.make_async_copy(w1_hbm.at[:, pl.ds(off, TF)],
                                     w1_v.at[j], sem.at[SEM_W1 + j])

    def w2_copy(c):
        off = pl.multiple_of(c * TS, TS)
        return pltpu.make_async_copy(w2_hbm.at[:, pl.ds(off, TS)],
                                     w2_v.at[c], sem.at[SEM_W2 + c])

    def wkv_copy():
        return pltpu.make_async_copy(wqkv_hbm.at[:, pl.ds(D, 2 * D)], wkv_v,
                                     sem.at[SEM_WKV])

    def wq_copy():
        return pltpu.make_async_copy(wqkv_hbm.at[:, pl.ds(0, D)], wq_v,
                                     sem.at[SEM_WQ])

    def wo_copy():
        return pltpu.make_async_copy(wo_hbm, wo_v, sem.at[SEM_WO])

    @pl.when(step < NS)
    def _stats():
        c = step

        @pl.when(c == 0)
        def _():
            x_copy(0).start()
            wkv_copy().start()
            z_ref[...] = jnp.zeros_like(z_ref)
            kv_ref[...] = jnp.zeros_like(kv_ref)

        @pl.when(c + 1 < NS)
        def _():
            x_copy(c + 1).start()

        @pl.when(c >= 1)
        def _():
            w1_copy(c - 1).start()

        x_copy(c).wait()
        off = pl.multiple_of(c * TS, TS)
        xb = x_v[pl.ds(off, TS), :]
        xc = xb.astype(jnp.float32)
        m = jnp.mean(xc, axis=-1, keepdims=True)
        xm = xc - m
        var = jnp.mean(xm * xm, axis=-1, keepdims=True)
        h = xm / jnp.sqrt(var + 1e-5)
        hT_ref[:, pl.ds(off, TS)] = h.T.astype(jnp.bfloat16)

        @pl.when(c == 0)
        def _():
            wkv_copy().wait()

        kv = jnp.dot(xb, wkv_v[...],
                     preferred_element_type=jnp.float32)
        pk = _phi(kv[:, :D])
        z_ref[...] += jnp.sum(pk, axis=0, keepdims=True)
        pkT = pk.T.astype(jnp.bfloat16)
        vb = kv[:, D:].astype(jnp.bfloat16)
        for g in range(NG):
            kv_ref[g] += jnp.dot(pkT[g * G:(g + 1) * G, :],
                                 vb[:, g * G:(g + 1) * G],
                                 preferred_element_type=jnp.float32)

        @pl.when(c == NS - 1)
        def _():
            ri = jax.lax.broadcasted_iota(jnp.int32, (G, G), 0) // DH
            ci = jax.lax.broadcasted_iota(jnp.int32, (G, G), 1) // DH
            mask = ri == ci
            z_row = z_ref[...]
            for g in range(NG):
                zb = jnp.broadcast_to(z_row[:, g * G:(g + 1) * G], (G, G)).T
                w_ref[g * G:(g + 1) * G, 0:G] = jnp.where(
                    mask, kv_ref[g], 0.0).astype(jnp.bfloat16)
                w_ref[g * G:(g + 1) * G, G:2 * G] = jnp.where(
                    mask, zb, 0.0).astype(jnp.bfloat16)

    @pl.when(jnp.logical_and(step >= NS, step < NS + NF))
    def _mixer1():
        j = step - NS
        w2_copy(j).start()

        @pl.when(j == 0)
        def _():
            wq_copy().start()
            wo_copy().start()

        @pl.when(j == NF - 1)
        def _():
            w2_copy(NS - 1).start()

        w1_copy(j).wait()
        off = pl.multiple_of(j * TF, TF)
        u = jnp.dot(hT_ref[...], w1_v[j],
                    preferred_element_type=jnp.float32)
        u = u + b1_ref[:, pl.ds(off, TF)].astype(jnp.float32)
        u_ref[:, pl.ds(off, TF)] = jax.nn.gelu(u, approximate=True).astype(
            jnp.bfloat16)

    @pl.when(step >= NS + NF)
    def _out():
        c = step - (NS + NF)

        @pl.when(c == 0)
        def _():
            wq_copy().wait()
            wo_copy().wait()

        w2_copy(c).wait()
        off = pl.multiple_of(c * TS, TS)
        xb = x_v[pl.ds(off, TS), :]
        xc = xb.astype(jnp.float32)
        gl = jnp.sum(xc * gw_ref[...].astype(jnp.float32), axis=-1,
                     keepdims=True)
        gate = jax.nn.sigmoid(gl)
        q = jnp.dot(xb, wq_v[...], preferred_element_type=jnp.float32)
        pq = _phi(q).astype(jnp.bfloat16)
        os = []
        for g in range(NG):
            nd = jnp.dot(pq[:, g * G:(g + 1) * G], w_ref[g * G:(g + 1) * G, :],
                         preferred_element_type=jnp.float32)
            os.append(nd[:, :G] / (nd[:, G:] + 1e-6))
        o = jnp.concatenate(os, axis=-1).astype(jnp.bfloat16)
        a = jnp.dot(o, wo_v[...], preferred_element_type=jnp.float32)
        y = jnp.dot(u_ref[...], w2_v[c],
                    preferred_element_type=jnp.float32)
        y = y + b2_ref[:, pl.ds(off, TS)].astype(jnp.float32)
        b = y.T
        o_ref[...] = (gate * a + (1.0 - gate) * b).astype(o_ref.dtype)


@jax.jit
def pallas_gated_mix__linear_attn_block__mixer_token_mlp__prompt_kernel(
    A_x: jax.Array,
    A_wqkv: jax.Array,
    A_wo: jax.Array,
    B_x: jax.Array,
    B_w1: jax.Array,
    B_b1: jax.Array,
    B_w2: jax.Array,
    B_b2: jax.Array,
    gate_w: jax.Array,
):
    x = A_x.reshape(S, D)
    b1 = B_b1.reshape(1, F)
    b2 = B_b2.reshape(1, S)
    gw = gate_w.reshape(1, D)
    nout = NS + NF

    out = pl.pallas_call(
        _kernel,
        grid=(NS + NF + NS,),
        in_specs=[
            pl.BlockSpec(memory_space=pl.ANY),
            pl.BlockSpec(memory_space=pl.ANY),
            pl.BlockSpec(memory_space=pl.ANY),
            pl.BlockSpec(memory_space=pl.ANY),
            pl.BlockSpec(memory_space=pl.ANY),
            pl.BlockSpec((1, F), lambda i: (0, 0)),
            pl.BlockSpec((1, S), lambda i: (0, 0)),
            pl.BlockSpec((1, D), lambda i: (0, 0)),
        ],
        out_specs=pl.BlockSpec((TS, D),
                               lambda i: (jnp.maximum(i - nout, 0), 0)),
        out_shape=jax.ShapeDtypeStruct((S, D), A_x.dtype),
        scratch_shapes=[
            pltpu.VMEM((S, D), jnp.bfloat16),
            pltpu.VMEM((D, 2 * D), jnp.bfloat16),
            pltpu.VMEM((D, D), jnp.bfloat16),
            pltpu.VMEM((D, D), jnp.bfloat16),
            pltpu.VMEM((NF, S, TF), jnp.bfloat16),
            pltpu.VMEM((NS, F, TS), jnp.bfloat16),
            pltpu.VMEM((D, S), jnp.bfloat16),
            pltpu.VMEM((D, F), jnp.bfloat16),
            pltpu.VMEM((NG, G, G), jnp.float32),
            pltpu.VMEM((1, D), jnp.float32),
            pltpu.VMEM((D, 2 * G), jnp.bfloat16),
            pltpu.SemaphoreType.DMA((NSEM,)),
        ],
        compiler_params=pltpu.CompilerParams(
            dimension_semantics=("arbitrary",),
            vmem_limit_bytes=64 * 1024 * 1024,
        ),
    )(x, A_wqkv, A_wo, B_w1, B_w2, b1, b2, gw)
    return out.reshape(1, S, D)
```

```python
import jax
import jax.numpy as jnp
import jax.experimental.pallas as pl
import jax.experimental.pallas.tpu as pltpu

S, D, F = 2048, 512, 1792
H = 32
DH = D // H
G = 128
NG = D // G
TF = 256
TS = 256
NF = F // TF
NS = S // TS

SEM_X = 0
SEM_W1 = SEM_X + NS
SEM_W2 = SEM_W1 + NF
SEM_WKV = SEM_W2 + NS
SEM_WQ = SEM_WKV + 1
SEM_WO = SEM_WQ + 1
NSEM = SEM_WO + 1


def _phi(t):
    return jnp.where(t > 0, t + 1.0, jnp.exp(t)) + 1e-6


def _kernel(x_hbm, wqkv_hbm, wo_hbm, w1_hbm, w2_hbm, b1_ref, b2_ref, gw_ref,
            o_ref,
            x_v, wkv_v, wq_v, wo_v, w1_v, w2_v, hT_ref, u_ref, kv_ref,
            w_ref, sem):
    step = pl.program_id(0)

    def x_copy(c):
        off = pl.multiple_of(c * TS, TS)
        return pltpu.make_async_copy(x_hbm.at[pl.ds(off, TS), :],
                                     x_v.at[pl.ds(off, TS), :],
                                     sem.at[SEM_X + c])

    def w1_copy(j):
        off = pl.multiple_of(j * TF, TF)
        return pltpu.make_async_copy(w1_hbm.at[:, pl.ds(off, TF)],
                                     w1_v.at[j], sem.at[SEM_W1 + j])

    def w2_copy(c):
        off = pl.multiple_of(c * TS, TS)
        return pltpu.make_async_copy(w2_hbm.at[:, pl.ds(off, TS)],
                                     w2_v.at[c], sem.at[SEM_W2 + c])

    def wkv_copy():
        return pltpu.make_async_copy(wqkv_hbm.at[:, pl.ds(D, 2 * D)], wkv_v,
                                     sem.at[SEM_WKV])

    def wq_copy():
        return pltpu.make_async_copy(wqkv_hbm.at[:, pl.ds(0, D)], wq_v,
                                     sem.at[SEM_WQ])

    def wo_copy():
        return pltpu.make_async_copy(wo_hbm, wo_v, sem.at[SEM_WO])

    @pl.when(step == 0)
    def _stats():
        x_copy(0).start()
        wkv_copy().start()
        z_row = jnp.zeros((1, D), jnp.float32)
        for c in range(NS):
            if c + 1 < NS:
                x_copy(c + 1).start()
            if c >= 1:
                w1_copy(c - 1).start()
            x_copy(c).wait()
            xb = x_v[c * TS:(c + 1) * TS, :]
            xc = xb.astype(jnp.float32)
            m = jnp.mean(xc, axis=-1, keepdims=True)
            xm = xc - m
            var = jnp.mean(xm * xm, axis=-1, keepdims=True)
            h = xm / jnp.sqrt(var + 1e-5)
            hT_ref[:, c * TS:(c + 1) * TS] = h.T.astype(jnp.bfloat16)
            if c == 0:
                wkv_copy().wait()
            kv = jnp.dot(xb, wkv_v[...],
                         preferred_element_type=jnp.float32)
            pk = _phi(kv[:, :D])
            z_row = z_row + jnp.sum(pk, axis=0, keepdims=True)
            pkT = pk.T.astype(jnp.bfloat16)
            vb = kv[:, D:].astype(jnp.bfloat16)
            for g in range(NG):
                part = jnp.dot(pkT[g * G:(g + 1) * G, :],
                               vb[:, g * G:(g + 1) * G],
                               preferred_element_type=jnp.float32)
                if c == 0:
                    kv_ref[g] = part
                else:
                    kv_ref[g] += part
        ri = jax.lax.broadcasted_iota(jnp.int32, (G, G), 0) // DH
        ci = jax.lax.broadcasted_iota(jnp.int32, (G, G), 1) // DH
        mask = ri == ci
        for g in range(NG):
            zb = jnp.broadcast_to(z_row[:, g * G:(g + 1) * G], (G, G)).T
            w_ref[g * G:(g + 1) * G, 0:G] = jnp.where(
                mask, kv_ref[g], 0.0).astype(jnp.bfloat16)
            w_ref[g * G:(g + 1) * G, G:2 * G] = jnp.where(
                mask, zb, 0.0).astype(jnp.bfloat16)

    @pl.when(jnp.logical_and(step >= 1, step < 1 + NF))
    def _mixer1():
        j = step - 1
        w2_copy(j).start()

        @pl.when(j == 0)
        def _():
            wq_copy().start()
            wo_copy().start()

        @pl.when(j == NF - 1)
        def _():
            w2_copy(NS - 1).start()

        w1_copy(j).wait()
        off = pl.multiple_of(j * TF, TF)
        u = jnp.dot(hT_ref[...], w1_v[j],
                    preferred_element_type=jnp.float32)
        u = u + b1_ref[:, pl.ds(off, TF)].astype(jnp.float32)
        u_ref[:, pl.ds(off, TF)] = jax.nn.gelu(u, approximate=True).astype(
            jnp.bfloat16)

    @pl.when(step >= 1 + NF)
    def _out():
        c = step - (1 + NF)

        @pl.when(c == 0)
        def _():
            wq_copy().wait()
            wo_copy().wait()

        w2_copy(c).wait()
        off = pl.multiple_of(c * TS, TS)
        xb = x_v[pl.ds(off, TS), :]
        xc = xb.astype(jnp.float32)
        gl = jnp.sum(xc * gw_ref[...].astype(jnp.float32), axis=-1,
                     keepdims=True)
        gate = jax.nn.sigmoid(gl)
        q = jnp.dot(xb, wq_v[...], preferred_element_type=jnp.float32)
        pq = _phi(q).astype(jnp.bfloat16)
        os = []
        for g in range(NG):
            nd = jnp.dot(pq[:, g * G:(g + 1) * G], w_ref[g * G:(g + 1) * G, :],
                         preferred_element_type=jnp.float32)
            os.append(nd[:, :G] / (nd[:, G:] + 1e-6))
        o = jnp.concatenate(os, axis=-1).astype(jnp.bfloat16)
        a = jnp.dot(o, wo_v[...], preferred_element_type=jnp.float32)
        y = jnp.dot(u_ref[...], w2_v[c],
                    preferred_element_type=jnp.float32)
        y = y + b2_ref[:, pl.ds(off, TS)].astype(jnp.float32)
        b = y.T
        o_ref[...] = (gate * a + (1.0 - gate) * b).astype(o_ref.dtype)


@jax.jit
def pallas_gated_mix__linear_attn_block__mixer_token_mlp__prompt_kernel(
    A_x: jax.Array,
    A_wqkv: jax.Array,
    A_wo: jax.Array,
    B_x: jax.Array,
    B_w1: jax.Array,
    B_b1: jax.Array,
    B_w2: jax.Array,
    B_b2: jax.Array,
    gate_w: jax.Array,
):
    x = A_x.reshape(S, D)
    b1 = B_b1.reshape(1, F)
    b2 = B_b2.reshape(1, S)
    gw = gate_w.reshape(1, D)
    nout = 1 + NF

    out = pl.pallas_call(
        _kernel,
        grid=(1 + NF + NS,),
        in_specs=[
            pl.BlockSpec(memory_space=pl.ANY),
            pl.BlockSpec(memory_space=pl.ANY),
            pl.BlockSpec(memory_space=pl.ANY),
            pl.BlockSpec(memory_space=pl.ANY),
            pl.BlockSpec(memory_space=pl.ANY),
            pl.BlockSpec((1, F), lambda i: (0, 0)),
            pl.BlockSpec((1, S), lambda i: (0, 0)),
            pl.BlockSpec((1, D), lambda i: (0, 0)),
        ],
        out_specs=pl.BlockSpec((TS, D),
                               lambda i: (jnp.maximum(i - nout, 0), 0)),
        out_shape=jax.ShapeDtypeStruct((S, D), A_x.dtype),
        scratch_shapes=[
            pltpu.VMEM((S, D), jnp.bfloat16),
            pltpu.VMEM((D, 2 * D), jnp.bfloat16),
            pltpu.VMEM((D, D), jnp.bfloat16),
            pltpu.VMEM((D, D), jnp.bfloat16),
            pltpu.VMEM((NF, S, TF), jnp.bfloat16),
            pltpu.VMEM((NS, F, TS), jnp.bfloat16),
            pltpu.VMEM((D, S), jnp.bfloat16),
            pltpu.VMEM((D, F), jnp.bfloat16),
            pltpu.VMEM((NG, G, G), jnp.float32),
            pltpu.VMEM((D, 2 * G), jnp.bfloat16),
            pltpu.SemaphoreType.DMA((NSEM,)),
        ],
        compiler_params=pltpu.CompilerParams(
            dimension_semantics=("arbitrary",),
            vmem_limit_bytes=64 * 1024 * 1024,
        ),
    )(x, A_wqkv, A_wo, B_w1, B_w2, b1, b2, gw)
    return out.reshape(1, S, D)
```

```python
import jax
import jax.numpy as jnp
import jax.experimental.pallas as pl
import jax.experimental.pallas.tpu as pltpu

S, D, F = 2048, 512, 1792
H = 32
DH = D // H
G = 128
NG = D // G
TF = 256
TS = 256
NF = F // TF
NS = S // TS

SEM_X = 0
SEM_W1 = SEM_X + NS
SEM_W2 = SEM_W1 + NF
SEM_WKV = SEM_W2 + NS
SEM_WQ = SEM_WKV + 1
SEM_WO = SEM_WQ + 1
NSEM = SEM_WO + 1


def _phi(t):
    return jnp.where(t > 0, t + 1.0, jnp.exp(t)) + 1e-6


def _kernel(x_hbm, wqkv_hbm, wo_hbm, w1_hbm, w2_hbm, b1_ref, b2_ref, gw_ref,
            o_ref,
            x_v, wkv_v, wq_v, wo_v, w1_v, w2_v, hT_ref, u_ref, kv_ref,
            w_ref, sem):
    step = pl.program_id(0)

    def x_copy(c):
        off = pl.multiple_of(c * TS, TS)
        return pltpu.make_async_copy(x_hbm.at[0, pl.ds(off, TS), :],
                                     x_v.at[pl.ds(off, TS), :],
                                     sem.at[SEM_X + c])

    def w1_copy(j):
        off = pl.multiple_of(j * TF, TF)
        return pltpu.make_async_copy(w1_hbm.at[:, pl.ds(off, TF)],
                                     w1_v.at[j], sem.at[SEM_W1 + j])

    def w2_copy(c):
        off = pl.multiple_of(c * TS, TS)
        return pltpu.make_async_copy(w2_hbm.at[:, pl.ds(off, TS)],
                                     w2_v.at[c], sem.at[SEM_W2 + c])

    def wkv_copy():
        return pltpu.make_async_copy(wqkv_hbm.at[:, pl.ds(D, 2 * D)], wkv_v,
                                     sem.at[SEM_WKV])

    def wq_copy():
        return pltpu.make_async_copy(wqkv_hbm.at[:, pl.ds(0, D)], wq_v,
                                     sem.at[SEM_WQ])

    def wo_copy():
        return pltpu.make_async_copy(wo_hbm, wo_v, sem.at[SEM_WO])

    @pl.when(step == 0)
    def _stats():
        x_copy(0).start()
        wkv_copy().start()
        z_row = jnp.zeros((1, D), jnp.float32)
        for c in range(NS):
            if c + 1 < NS:
                x_copy(c + 1).start()
            if c >= 1:
                w1_copy(c - 1).start()
            x_copy(c).wait()
            xb = x_v[c * TS:(c + 1) * TS, :]
            xc = xb.astype(jnp.float32)
            m = jnp.mean(xc, axis=-1, keepdims=True)
            xm = xc - m
            var = jnp.mean(xm * xm, axis=-1, keepdims=True)
            h = xm / jnp.sqrt(var + 1e-5)
            hT_ref[:, c * TS:(c + 1) * TS] = h.T.astype(jnp.bfloat16)
            if c == 0:
                wkv_copy().wait()
            kv = jnp.dot(xb, wkv_v[...],
                         preferred_element_type=jnp.float32)
            pk = _phi(kv[:, :D])
            z_row = z_row + jnp.sum(pk, axis=0, keepdims=True)
            pkT = pk.T.astype(jnp.bfloat16)
            vb = kv[:, D:].astype(jnp.bfloat16)
            for g in range(NG):
                part = jnp.dot(pkT[g * G:(g + 1) * G, :],
                               vb[:, g * G:(g + 1) * G],
                               preferred_element_type=jnp.float32)
                if c == 0:
                    kv_ref[g] = part
                else:
                    kv_ref[g] += part
        ri = jax.lax.broadcasted_iota(jnp.int32, (G, G), 0) // DH
        ci = jax.lax.broadcasted_iota(jnp.int32, (G, G), 1) // DH
        mask = ri == ci
        for g in range(NG):
            zb = jnp.broadcast_to(z_row[:, g * G:(g + 1) * G], (G, G)).T
            w_ref[g * G:(g + 1) * G, 0:G] = jnp.where(
                mask, kv_ref[g], 0.0).astype(jnp.bfloat16)
            w_ref[g * G:(g + 1) * G, G:2 * G] = jnp.where(
                mask, zb, 0.0).astype(jnp.bfloat16)

    @pl.when(jnp.logical_and(step >= 1, step < 1 + NF))
    def _mixer1():
        j = step - 1
        w2_copy(j).start()

        @pl.when(j == 0)
        def _():
            wq_copy().start()
            wo_copy().start()

        @pl.when(j == NF - 1)
        def _():
            w2_copy(NS - 1).start()

        w1_copy(j).wait()
        off = pl.multiple_of(j * TF, TF)
        u = jnp.dot(hT_ref[...], w1_v[j],
                    preferred_element_type=jnp.float32)
        u = u + b1_ref[pl.ds(off, TF)].reshape(1, TF).astype(jnp.float32)
        u_ref[:, pl.ds(off, TF)] = jax.nn.gelu(u, approximate=True).astype(
            jnp.bfloat16)

    @pl.when(step >= 1 + NF)
    def _out():
        c = step - (1 + NF)

        @pl.when(c == 0)
        def _():
            wq_copy().wait()
            wo_copy().wait()

        w2_copy(c).wait()
        off = pl.multiple_of(c * TS, TS)
        xb = x_v[pl.ds(off, TS), :]
        xc = xb.astype(jnp.float32)
        y = jnp.dot(u_ref[...], w2_v[c],
                    preferred_element_type=jnp.float32)
        y = y + b2_ref[pl.ds(off, TS)].reshape(1, TS).astype(jnp.float32)
        b = y.T
        gl = jnp.sum(xc * gw_ref[...].reshape(1, D).astype(jnp.float32), axis=-1,
                     keepdims=True)
        gate = jax.nn.sigmoid(gl)
        q = jnp.dot(xb, wq_v[...], preferred_element_type=jnp.float32)
        pq = _phi(q).astype(jnp.bfloat16)
        os = []
        for g in range(NG):
            nd = jnp.dot(pq[:, g * G:(g + 1) * G], w_ref[g * G:(g + 1) * G, :],
                         preferred_element_type=jnp.float32)
            os.append(nd[:, :G] / (nd[:, G:] + 1e-6))
        o = jnp.concatenate(os, axis=-1).astype(jnp.bfloat16)
        a = jnp.dot(o, wo_v[...], preferred_element_type=jnp.float32)
        o_ref[...] = (gate * a + (1.0 - gate) * b).astype(o_ref.dtype)


@jax.jit
def pallas_gated_mix__linear_attn_block__mixer_token_mlp__prompt_kernel(
    A_x: jax.Array,
    A_wqkv: jax.Array,
    A_wo: jax.Array,
    B_x: jax.Array,
    B_w1: jax.Array,
    B_b1: jax.Array,
    B_w2: jax.Array,
    B_b2: jax.Array,
    gate_w: jax.Array,
):
    nout = 1 + NF

    out = pl.pallas_call(
        _kernel,
        grid=(1 + NF + NS,),
        in_specs=[
            pl.BlockSpec(memory_space=pl.ANY),
            pl.BlockSpec(memory_space=pl.ANY),
            pl.BlockSpec(memory_space=pl.ANY),
            pl.BlockSpec(memory_space=pl.ANY),
            pl.BlockSpec(memory_space=pl.ANY),
            pl.BlockSpec((F,), lambda i: (0,)),
            pl.BlockSpec((S,), lambda i: (0,)),
            pl.BlockSpec((D,), lambda i: (0,)),
        ],
        out_specs=pl.BlockSpec((None, TS, D),
                               lambda i: (0, jnp.maximum(i - nout, 0), 0)),
        out_shape=jax.ShapeDtypeStruct((1, S, D), A_x.dtype),
        scratch_shapes=[
            pltpu.VMEM((S, D), jnp.bfloat16),
            pltpu.VMEM((D, 2 * D), jnp.bfloat16),
            pltpu.VMEM((D, D), jnp.bfloat16),
            pltpu.VMEM((D, D), jnp.bfloat16),
            pltpu.VMEM((NF, S, TF), jnp.bfloat16),
            pltpu.VMEM((NS, F, TS), jnp.bfloat16),
            pltpu.VMEM((D, S), jnp.bfloat16),
            pltpu.VMEM((D, F), jnp.bfloat16),
            pltpu.VMEM((NG, G, G), jnp.float32),
            pltpu.VMEM((D, 2 * G), jnp.bfloat16),
            pltpu.SemaphoreType.DMA((NSEM,)),
        ],
        compiler_params=pltpu.CompilerParams(
            dimension_semantics=("arbitrary",),
            vmem_limit_bytes=64 * 1024 * 1024,
        ),
    )(A_x, A_wqkv, A_wo, B_w1, B_w2, B_b1, B_b2, gate_w)
    return out
```

```python
import jax
import jax.numpy as jnp
import jax.experimental.pallas as pl
import jax.experimental.pallas.tpu as pltpu

S, D, F = 2048, 512, 1792
H = 32
DH = D // H
G = 128
NG = D // G
TF = 256
TS = 256
NF = F // TF
NS = S // TS

SEM_X = 0
SEM_W1 = SEM_X + NS
SEM_W2 = SEM_W1 + NF
SEM_WKV = SEM_W2 + NS
SEM_WQ = SEM_WKV + 1
SEM_WO = SEM_WQ + 1
NSEM = SEM_WO + 1


def _phi(t):
    return jnp.where(t > 0, t + 1.0, jnp.exp(t)) + 1e-6


def _kernel(x_hbm, wqkv_hbm, wo_hbm, w1_hbm, w2_hbm, b1_ref, b2_ref, gw_ref,
            o_ref,
            x_v, wkv_v, wq_v, wo_v, w1_v, w2_v, hT_ref, u_ref, kv_ref,
            w_ref, sem):
    step = pl.program_id(0)

    def x_copy(c):
        off = pl.multiple_of(c * TS, TS)
        return pltpu.make_async_copy(x_hbm.at[0, pl.ds(off, TS), :],
                                     x_v.at[pl.ds(off, TS), :],
                                     sem.at[SEM_X + c])

    def xr_copy():
        return pltpu.make_async_copy(x_hbm.at[0, pl.ds(2 * TS, S - 2 * TS), :],
                                     x_v.at[pl.ds(2 * TS, S - 2 * TS), :],
                                     sem.at[SEM_X + 2])

    def w1_copy(j):
        off = pl.multiple_of(j * TF, TF)
        return pltpu.make_async_copy(w1_hbm.at[:, pl.ds(off, TF)],
                                     w1_v.at[j], sem.at[SEM_W1 + j])

    def w2_copy(c):
        off = pl.multiple_of(c * TS, TS)
        return pltpu.make_async_copy(w2_hbm.at[:, pl.ds(off, TS)],
                                     w2_v.at[c], sem.at[SEM_W2 + c])

    def wkv_copy():
        return pltpu.make_async_copy(wqkv_hbm.at[:, pl.ds(D, 2 * D)], wkv_v,
                                     sem.at[SEM_WKV])

    def wq_copy():
        return pltpu.make_async_copy(wqkv_hbm.at[:, pl.ds(0, D)], wq_v,
                                     sem.at[SEM_WQ])

    def wo_copy():
        return pltpu.make_async_copy(wo_hbm, wo_v, sem.at[SEM_WO])

    @pl.when(step == 0)
    def _stats():
        x_copy(0).start()
        wkv_copy().start()
        x_copy(1).start()
        z_row = jnp.zeros((1, D), jnp.float32)
        for c in range(NS):
            if c == 0:
                x_copy(0).wait()
                xr_copy().start()
            elif c == 1:
                x_copy(1).wait()
                for j in range(NF):
                    w1_copy(j).start()
            elif c == 2:
                xr_copy().wait()
            xb = x_v[c * TS:(c + 1) * TS, :]
            xc = xb.astype(jnp.float32)
            m = jnp.mean(xc, axis=-1, keepdims=True)
            xm = xc - m
            var = jnp.mean(xm * xm, axis=-1, keepdims=True)
            h = xm / jnp.sqrt(var + 1e-5)
            hT_ref[:, c * TS:(c + 1) * TS] = h.T.astype(jnp.bfloat16)
            if c == 0:
                wkv_copy().wait()
            kv = jnp.dot(xb, wkv_v[...],
                         preferred_element_type=jnp.float32)
            pk = _phi(kv[:, :D])
            z_row = z_row + jnp.sum(pk, axis=0, keepdims=True)
            pkT = pk.T.astype(jnp.bfloat16)
            vb = kv[:, D:].astype(jnp.bfloat16)
            for g in range(NG):
                part = jnp.dot(pkT[g * G:(g + 1) * G, :],
                               vb[:, g * G:(g + 1) * G],
                               preferred_element_type=jnp.float32)
                if c == 0:
                    kv_ref[g] = part
                else:
                    kv_ref[g] += part
        ri = jax.lax.broadcasted_iota(jnp.int32, (G, G), 0) // DH
        ci = jax.lax.broadcasted_iota(jnp.int32, (G, G), 1) // DH
        mask = ri == ci
        for g in range(NG):
            zb = jnp.broadcast_to(z_row[:, g * G:(g + 1) * G], (G, G)).T
            w_ref[g * G:(g + 1) * G, 0:G] = jnp.where(
                mask, kv_ref[g], 0.0).astype(jnp.bfloat16)
            w_ref[g * G:(g + 1) * G, G:2 * G] = jnp.where(
                mask, zb, 0.0).astype(jnp.bfloat16)

    @pl.when(jnp.logical_and(step >= 1, step < 1 + NF))
    def _mixer1():
        j = step - 1
        w2_copy(j).start()

        @pl.when(j == 0)
        def _():
            wq_copy().start()
            wo_copy().start()

        @pl.when(j == NF - 1)
        def _():
            w2_copy(NS - 1).start()

        w1_copy(j).wait()
        off = pl.multiple_of(j * TF, TF)
        u = jnp.dot(hT_ref[...], w1_v[j],
                    preferred_element_type=jnp.float32)
        u = u + b1_ref[pl.ds(off, TF)].reshape(1, TF).astype(jnp.float32)
        u_ref[:, pl.ds(off, TF)] = jax.nn.gelu(u, approximate=True).astype(
            jnp.bfloat16)

    @pl.when(step >= 1 + NF)
    def _out():
        c = step - (1 + NF)

        @pl.when(c == 0)
        def _():
            wq_copy().wait()
            wo_copy().wait()

        w2_copy(c).wait()
        off = pl.multiple_of(c * TS, TS)
        xb = x_v[pl.ds(off, TS), :]
        xc = xb.astype(jnp.float32)
        y = jnp.dot(u_ref[...], w2_v[c],
                    preferred_element_type=jnp.float32)
        y = y + b2_ref[pl.ds(off, TS)].reshape(1, TS).astype(jnp.float32)
        b = y.T
        gl = jnp.sum(xc * gw_ref[...].reshape(1, D).astype(jnp.float32), axis=-1,
                     keepdims=True)
        gate = jax.nn.sigmoid(gl)
        q = jnp.dot(xb, wq_v[...], preferred_element_type=jnp.float32)
        pq = _phi(q).astype(jnp.bfloat16)
        os = []
        for g in range(NG):
            nd = jnp.dot(pq[:, g * G:(g + 1) * G], w_ref[g * G:(g + 1) * G, :],
                         preferred_element_type=jnp.float32)
            os.append(nd[:, :G] / (nd[:, G:] + 1e-6))
        o = jnp.concatenate(os, axis=-1).astype(jnp.bfloat16)
        a = jnp.dot(o, wo_v[...], preferred_element_type=jnp.float32)
        o_ref[...] = (gate * a + (1.0 - gate) * b).astype(o_ref.dtype)


@jax.jit
def pallas_gated_mix__linear_attn_block__mixer_token_mlp__prompt_kernel(
    A_x: jax.Array,
    A_wqkv: jax.Array,
    A_wo: jax.Array,
    B_x: jax.Array,
    B_w1: jax.Array,
    B_b1: jax.Array,
    B_w2: jax.Array,
    B_b2: jax.Array,
    gate_w: jax.Array,
):
    nout = 1 + NF

    out = pl.pallas_call(
        _kernel,
        grid=(1 + NF + NS,),
        in_specs=[
            pl.BlockSpec(memory_space=pl.ANY),
            pl.BlockSpec(memory_space=pl.ANY),
            pl.BlockSpec(memory_space=pl.ANY),
            pl.BlockSpec(memory_space=pl.ANY),
            pl.BlockSpec(memory_space=pl.ANY),
            pl.BlockSpec((F,), lambda i: (0,)),
            pl.BlockSpec((S,), lambda i: (0,)),
            pl.BlockSpec((D,), lambda i: (0,)),
        ],
        out_specs=pl.BlockSpec((None, TS, D),
                               lambda i: (0, jnp.maximum(i - nout, 0), 0)),
        out_shape=jax.ShapeDtypeStruct((1, S, D), A_x.dtype),
        scratch_shapes=[
            pltpu.VMEM((S, D), jnp.bfloat16),
            pltpu.VMEM((D, 2 * D), jnp.bfloat16),
            pltpu.VMEM((D, D), jnp.bfloat16),
            pltpu.VMEM((D, D), jnp.bfloat16),
            pltpu.VMEM((NF, S, TF), jnp.bfloat16),
            pltpu.VMEM((NS, F, TS), jnp.bfloat16),
            pltpu.VMEM((D, S), jnp.bfloat16),
            pltpu.VMEM((D, F), jnp.bfloat16),
            pltpu.VMEM((NG, G, G), jnp.float32),
            pltpu.VMEM((D, 2 * G), jnp.bfloat16),
            pltpu.SemaphoreType.DMA((NSEM,)),
        ],
        compiler_params=pltpu.CompilerParams(
            dimension_semantics=("arbitrary",),
            vmem_limit_bytes=64 * 1024 * 1024,
        ),
    )(A_x, A_wqkv, A_wo, B_w1, B_w2, B_b1, B_b2, gate_w)
    return out
```

```python
import jax
import jax.numpy as jnp
import jax.experimental.pallas as pl
import jax.experimental.pallas.tpu as pltpu

S, D, F = 2048, 512, 1792
H = 32
DH = D // H
G = 128
NG = D // G
TF = 256
TS = 256
NF = F // TF
NS = S // TS

SEM_X = 0
SEM_W1 = SEM_X + NS
SEM_W2 = SEM_W1 + NF
SEM_WKV = SEM_W2 + NS
SEM_WQ = SEM_WKV + 1
SEM_WO = SEM_WQ + 1
NSEM = SEM_WO + 1


def _phi(t):
    return jnp.where(t > 0, t + 1.0, jnp.exp(t)) + 1e-6


def _kernel(x_hbm, wqkv_hbm, wo_hbm, w1_hbm, w2_hbm, b1_ref, b2_ref, gw_ref,
            o_ref,
            x_v, wkv_v, wq_v, wo_v, w1_v, w2_v, hT_ref, u_ref, kv_ref,
            w_ref, sem):
    step = pl.program_id(0)

    def x_copy(c):
        off = pl.multiple_of(c * TS, TS)
        return pltpu.make_async_copy(x_hbm.at[0, pl.ds(off, TS), :],
                                     x_v.at[pl.ds(off, TS), :],
                                     sem.at[SEM_X + c])

    def xr_copy():
        return pltpu.make_async_copy(x_hbm.at[0, pl.ds(2 * TS, S - 2 * TS), :],
                                     x_v.at[pl.ds(2 * TS, S - 2 * TS), :],
                                     sem.at[SEM_X + 2])

    def w1_copy(j):
        off = pl.multiple_of(j * TF, TF)
        return pltpu.make_async_copy(w1_hbm.at[:, pl.ds(off, TF)],
                                     w1_v.at[j], sem.at[SEM_W1 + j])

    def w2_copy(c):
        off = pl.multiple_of(c * TS, TS)
        return pltpu.make_async_copy(w2_hbm.at[:, pl.ds(off, TS)],
                                     w2_v.at[c], sem.at[SEM_W2 + c])

    def wkv_copy():
        return pltpu.make_async_copy(wqkv_hbm.at[:, pl.ds(D, 2 * D)], wkv_v,
                                     sem.at[SEM_WKV])

    def wq_copy():
        return pltpu.make_async_copy(wqkv_hbm.at[:, pl.ds(0, D)], wq_v,
                                     sem.at[SEM_WQ])

    def wo_copy():
        return pltpu.make_async_copy(wo_hbm, wo_v, sem.at[SEM_WO])

    @pl.when(step == 0)
    def _stats():
        x_copy(0).start()
        wkv_copy().start()
        x_copy(1).start()
        z_row = jnp.zeros((1, D), jnp.float32)
        for c in range(NS):
            if c == 0:
                x_copy(0).wait()
                xr_copy().start()
            elif c == 1:
                x_copy(1).wait()
                for j in range(NF):
                    w1_copy(j).start()
            elif c == 2:
                xr_copy().wait()
            xb = x_v[c * TS:(c + 1) * TS, :]
            xc = xb.astype(jnp.float32)
            m = jnp.mean(xc, axis=-1, keepdims=True)
            xm = xc - m
            var = jnp.mean(xm * xm, axis=-1, keepdims=True)
            h = xm / jnp.sqrt(var + 1e-5)
            hT_ref[:, c * TS:(c + 1) * TS] = h.T.astype(jnp.bfloat16)
            if c == 0:
                wkv_copy().wait()
            kv = jnp.dot(xb, wkv_v[...],
                         preferred_element_type=jnp.float32)
            pk = _phi(kv[:, :D])
            z_row = z_row + jnp.sum(pk, axis=0, keepdims=True)
            pkT = pk.T.astype(jnp.bfloat16)
            vb = kv[:, D:].astype(jnp.bfloat16)
            for g in range(NG):
                part = jnp.dot(pkT[g * G:(g + 1) * G, :],
                               vb[:, g * G:(g + 1) * G],
                               preferred_element_type=jnp.float32)
                if c == 0:
                    kv_ref[g] = part
                else:
                    kv_ref[g] += part
        ri = jax.lax.broadcasted_iota(jnp.int32, (G, G), 0) // DH
        ci = jax.lax.broadcasted_iota(jnp.int32, (G, G), 1) // DH
        mask = ri == ci
        for g in range(NG):
            zb = jnp.broadcast_to(z_row[:, g * G:(g + 1) * G], (G, G)).T
            w_ref[g * G:(g + 1) * G, 0:G] = jnp.where(
                mask, kv_ref[g], 0.0).astype(jnp.bfloat16)
            w_ref[g * G:(g + 1) * G, G:2 * G] = jnp.where(
                mask, zb, 0.0).astype(jnp.bfloat16)

    @pl.when(step == 1)
    def _mixer1():
        for c in range(NS):
            w2_copy(c).start()
        wq_copy().start()
        wo_copy().start()
        for j in range(NF):
            w1_copy(j).wait()
        for j in range(NF):
            u = jnp.dot(hT_ref[...], w1_v[j],
                        preferred_element_type=jnp.float32)
            u = u + b1_ref[j * TF:(j + 1) * TF].reshape(1, TF).astype(
                jnp.float32)
            u_ref[:, j * TF:(j + 1) * TF] = jax.nn.gelu(
                u, approximate=True).astype(jnp.bfloat16)

    @pl.when(step >= 2)
    def _out():
        c = step - 2

        @pl.when(c == 0)
        def _():
            wq_copy().wait()
            wo_copy().wait()

        w2_copy(c).wait()
        off = pl.multiple_of(c * TS, TS)
        xb = x_v[pl.ds(off, TS), :]
        xc = xb.astype(jnp.float32)
        y = jnp.dot(u_ref[...], w2_v[c],
                    preferred_element_type=jnp.float32)
        y = y + b2_ref[pl.ds(off, TS)].reshape(1, TS).astype(jnp.float32)
        b = y.T
        gl = jnp.sum(xc * gw_ref[...].reshape(1, D).astype(jnp.float32), axis=-1,
                     keepdims=True)
        gate = jax.nn.sigmoid(gl)
        q = jnp.dot(xb, wq_v[...], preferred_element_type=jnp.float32)
        pq = _phi(q).astype(jnp.bfloat16)
        os = []
        for g in range(NG):
            nd = jnp.dot(pq[:, g * G:(g + 1) * G], w_ref[g * G:(g + 1) * G, :],
                         preferred_element_type=jnp.float32)
            os.append(nd[:, :G] / (nd[:, G:] + 1e-6))
        o = jnp.concatenate(os, axis=-1).astype(jnp.bfloat16)
        a = jnp.dot(o, wo_v[...], preferred_element_type=jnp.float32)
        o_ref[...] = (gate * a + (1.0 - gate) * b).astype(o_ref.dtype)


@jax.jit
def pallas_gated_mix__linear_attn_block__mixer_token_mlp__prompt_kernel(
    A_x: jax.Array,
    A_wqkv: jax.Array,
    A_wo: jax.Array,
    B_x: jax.Array,
    B_w1: jax.Array,
    B_b1: jax.Array,
    B_w2: jax.Array,
    B_b2: jax.Array,
    gate_w: jax.Array,
):
    nout = 2

    out = pl.pallas_call(
        _kernel,
        grid=(2 + NS,),
        in_specs=[
            pl.BlockSpec(memory_space=pl.ANY),
            pl.BlockSpec(memory_space=pl.ANY),
            pl.BlockSpec(memory_space=pl.ANY),
            pl.BlockSpec(memory_space=pl.ANY),
            pl.BlockSpec(memory_space=pl.ANY),
            pl.BlockSpec((F,), lambda i: (0,)),
            pl.BlockSpec((S,), lambda i: (0,)),
            pl.BlockSpec((D,), lambda i: (0,)),
        ],
        out_specs=pl.BlockSpec((None, TS, D),
                               lambda i: (0, jnp.maximum(i - nout, 0), 0)),
        out_shape=jax.ShapeDtypeStruct((1, S, D), A_x.dtype),
        scratch_shapes=[
            pltpu.VMEM((S, D), jnp.bfloat16),
            pltpu.VMEM((D, 2 * D), jnp.bfloat16),
            pltpu.VMEM((D, D), jnp.bfloat16),
            pltpu.VMEM((D, D), jnp.bfloat16),
            pltpu.VMEM((NF, S, TF), jnp.bfloat16),
            pltpu.VMEM((NS, F, TS), jnp.bfloat16),
            pltpu.VMEM((D, S), jnp.bfloat16),
            pltpu.VMEM((D, F), jnp.bfloat16),
            pltpu.VMEM((NG, G, G), jnp.float32),
            pltpu.VMEM((D, 2 * G), jnp.bfloat16),
            pltpu.SemaphoreType.DMA((NSEM,)),
        ],
        compiler_params=pltpu.CompilerParams(
            dimension_semantics=("arbitrary",),
            vmem_limit_bytes=64 * 1024 * 1024,
        ),
    )(A_x, A_wqkv, A_wo, B_w1, B_w2, B_b1, B_b2, gate_w)
    return out
```

```python
import jax
import jax.numpy as jnp
import jax.experimental.pallas as pl
import jax.experimental.pallas.tpu as pltpu

S, D, F = 2048, 512, 1792
H = 32
DH = D // H
G = 128
NG = D // G
TF = 256
TS = 256
NF = F // TF
NS = S // TS
CPS = 2

SEM_X = 0
SEM_W1 = SEM_X + NS
SEM_W2 = SEM_W1 + NF
SEM_WKV = SEM_W2 + NS
SEM_WQ = SEM_WKV + 1
SEM_WO = SEM_WQ + 1
NSEM = SEM_WO + 1


def _phi(t):
    return jnp.where(t > 0, t + 1.0, jnp.exp(t)) + 1e-6


def _kernel(x_hbm, wqkv_hbm, wo_hbm, w1_hbm, w2_hbm, b1_ref, b2_ref, gw_ref,
            o_ref,
            x_v, wkv_v, wq_v, wo_v, w1_v, w2_v, hT_ref, u_ref, kv_ref,
            w_ref, sem):
    step = pl.program_id(0)

    def x_copy(c):
        off = pl.multiple_of(c * TS, TS)
        return pltpu.make_async_copy(x_hbm.at[0, pl.ds(off, TS), :],
                                     x_v.at[pl.ds(off, TS), :],
                                     sem.at[SEM_X + c])

    def xr_copy():
        return pltpu.make_async_copy(x_hbm.at[0, pl.ds(2 * TS, S - 2 * TS), :],
                                     x_v.at[pl.ds(2 * TS, S - 2 * TS), :],
                                     sem.at[SEM_X + 2])

    def w1_copy(j):
        off = pl.multiple_of(j * TF, TF)
        return pltpu.make_async_copy(w1_hbm.at[:, pl.ds(off, TF)],
                                     w1_v.at[j], sem.at[SEM_W1 + j])

    def w2_copy(c):
        off = pl.multiple_of(c * TS, TS)
        return pltpu.make_async_copy(w2_hbm.at[:, pl.ds(off, TS)],
                                     w2_v.at[c], sem.at[SEM_W2 + c])

    def wkv_copy():
        return pltpu.make_async_copy(wqkv_hbm.at[:, pl.ds(D, 2 * D)], wkv_v,
                                     sem.at[SEM_WKV])

    def wq_copy():
        return pltpu.make_async_copy(wqkv_hbm.at[:, pl.ds(0, D)], wq_v,
                                     sem.at[SEM_WQ])

    def wo_copy():
        return pltpu.make_async_copy(wo_hbm, wo_v, sem.at[SEM_WO])

    @pl.when(step == 0)
    def _stats():
        x_copy(0).start()
        wkv_copy().start()
        x_copy(1).start()
        z_row = jnp.zeros((1, D), jnp.float32)
        for c in range(NS):
            if c == 0:
                x_copy(0).wait()
                xr_copy().start()
            elif c == 1:
                x_copy(1).wait()
                for j in range(NF):
                    w1_copy(j).start()
            elif c == 2:
                xr_copy().wait()
            xb = x_v[c * TS:(c + 1) * TS, :]
            xc = xb.astype(jnp.float32)
            m = jnp.mean(xc, axis=-1, keepdims=True)
            xm = xc - m
            var = jnp.mean(xm * xm, axis=-1, keepdims=True)
            h = xm / jnp.sqrt(var + 1e-5)
            hT_ref[:, c * TS:(c + 1) * TS] = h.T.astype(jnp.bfloat16)
            if c == 0:
                wkv_copy().wait()
            kv = jnp.dot(xb, wkv_v[...],
                         preferred_element_type=jnp.float32)
            pk = _phi(kv[:, :D])
            z_row = z_row + jnp.sum(pk, axis=0, keepdims=True)
            pkT = pk.T.astype(jnp.bfloat16)
            vb = kv[:, D:].astype(jnp.bfloat16)
            for g in range(NG):
                part = jnp.dot(pkT[g * G:(g + 1) * G, :],
                               vb[:, g * G:(g + 1) * G],
                               preferred_element_type=jnp.float32)
                if c == 0:
                    kv_ref[g] = part
                else:
                    kv_ref[g] += part
        ri = jax.lax.broadcasted_iota(jnp.int32, (G, G), 0) // DH
        ci = jax.lax.broadcasted_iota(jnp.int32, (G, G), 1) // DH
        mask = ri == ci
        for g in range(NG):
            zb = jnp.broadcast_to(z_row[:, g * G:(g + 1) * G], (G, G)).T
            w_ref[g * G:(g + 1) * G, 0:G] = jnp.where(
                mask, kv_ref[g], 0.0).astype(jnp.bfloat16)
            w_ref[g * G:(g + 1) * G, G:2 * G] = jnp.where(
                mask, zb, 0.0).astype(jnp.bfloat16)

    @pl.when(step == 1)
    def _mixer1():
        for c in range(NS):
            w2_copy(c).start()
        wq_copy().start()
        wo_copy().start()
        for j in range(NF):
            w1_copy(j).wait()
        for j in range(NF):
            u = jnp.dot(hT_ref[...], w1_v[j],
                        preferred_element_type=jnp.float32)
            u = u + b1_ref[j * TF:(j + 1) * TF].reshape(1, TF).astype(
                jnp.float32)
            u_ref[:, j * TF:(j + 1) * TF] = jax.nn.gelu(
                u, approximate=True).astype(jnp.bfloat16)

    @pl.when(step >= 2)
    def _out():
        cs = step - 2

        @pl.when(cs == 0)
        def _():
            wq_copy().wait()
            wo_copy().wait()

        for r in range(CPS):
            w2_copy(cs * CPS + r).wait()
        for r in range(CPS):
            c = cs * CPS + r
            off = pl.multiple_of(c * TS, TS)
            xb = x_v[pl.ds(off, TS), :]
            xc = xb.astype(jnp.float32)
            y = jnp.dot(u_ref[...], w2_v[c],
                        preferred_element_type=jnp.float32)
            y = y + b2_ref[pl.ds(off, TS)].reshape(1, TS).astype(jnp.float32)
            b = y.T
            gl = jnp.sum(xc * gw_ref[...].reshape(1, D).astype(jnp.float32),
                         axis=-1, keepdims=True)
            gate = jax.nn.sigmoid(gl)
            q = jnp.dot(xb, wq_v[...], preferred_element_type=jnp.float32)
            pq = _phi(q).astype(jnp.bfloat16)
            os = []
            for g in range(NG):
                nd = jnp.dot(pq[:, g * G:(g + 1) * G],
                             w_ref[g * G:(g + 1) * G, :],
                             preferred_element_type=jnp.float32)
                os.append(nd[:, :G] / (nd[:, G:] + 1e-6))
            o = jnp.concatenate(os, axis=-1).astype(jnp.bfloat16)
            a = jnp.dot(o, wo_v[...], preferred_element_type=jnp.float32)
            o_ref[r * TS:(r + 1) * TS, :] = (
                gate * a + (1.0 - gate) * b).astype(o_ref.dtype)


@jax.jit
def pallas_gated_mix__linear_attn_block__mixer_token_mlp__prompt_kernel(
    A_x: jax.Array,
    A_wqkv: jax.Array,
    A_wo: jax.Array,
    B_x: jax.Array,
    B_w1: jax.Array,
    B_b1: jax.Array,
    B_w2: jax.Array,
    B_b2: jax.Array,
    gate_w: jax.Array,
):
    nout = 2

    out = pl.pallas_call(
        _kernel,
        grid=(2 + NS // CPS,),
        in_specs=[
            pl.BlockSpec(memory_space=pl.ANY),
            pl.BlockSpec(memory_space=pl.ANY),
            pl.BlockSpec(memory_space=pl.ANY),
            pl.BlockSpec(memory_space=pl.ANY),
            pl.BlockSpec(memory_space=pl.ANY),
            pl.BlockSpec((F,), lambda i: (0,)),
            pl.BlockSpec((S,), lambda i: (0,)),
            pl.BlockSpec((D,), lambda i: (0,)),
        ],
        out_specs=pl.BlockSpec((None, CPS * TS, D),
                               lambda i: (0, jnp.maximum(i - nout, 0), 0)),
        out_shape=jax.ShapeDtypeStruct((1, S, D), A_x.dtype),
        scratch_shapes=[
            pltpu.VMEM((S, D), jnp.bfloat16),
            pltpu.VMEM((D, 2 * D), jnp.bfloat16),
            pltpu.VMEM((D, D), jnp.bfloat16),
            pltpu.VMEM((D, D), jnp.bfloat16),
            pltpu.VMEM((NF, S, TF), jnp.bfloat16),
            pltpu.VMEM((NS, F, TS), jnp.bfloat16),
            pltpu.VMEM((D, S), jnp.bfloat16),
            pltpu.VMEM((D, F), jnp.bfloat16),
            pltpu.VMEM((NG, G, G), jnp.float32),
            pltpu.VMEM((D, 2 * G), jnp.bfloat16),
            pltpu.SemaphoreType.DMA((NSEM,)),
        ],
        compiler_params=pltpu.CompilerParams(
            dimension_semantics=("arbitrary",),
            vmem_limit_bytes=64 * 1024 * 1024,
        ),
    )(A_x, A_wqkv, A_wo, B_w1, B_w2, B_b1, B_b2, gate_w)
    return out
```

```python
import jax
import jax.numpy as jnp
import jax.experimental.pallas as pl
import jax.experimental.pallas.tpu as pltpu

S, D, F = 2048, 512, 1792
H = 32
DH = D // H
G = 128
NG = D // G
TF = 256
TS = 256
NF = F // TF
NS = S // TS
CPS = 2

SEM_X = 0
SEM_W1 = SEM_X + NS
SEM_W2 = SEM_W1 + NF
SEM_WKV = SEM_W2 + NS
SEM_WQ = SEM_WKV + 1
SEM_WO = SEM_WQ + 1
NSEM = SEM_WO + 1


def _phi(t):
    return jnp.where(t > 0, t + 1.0, jnp.exp(t)) + 1e-6


def _kernel(x_hbm, wqkv_hbm, wo_hbm, w1_hbm, w2_hbm, b1_ref, b2_ref, gw_ref,
            o_ref,
            x_v, wkv_v, wq_v, wo_v, w1_v, w2_v, hT_ref, u_ref, kv_ref,
            w_ref, sem):
    step = pl.program_id(0)

    def x_copy(c):
        off = pl.multiple_of(c * TS, TS)
        return pltpu.make_async_copy(x_hbm.at[0, pl.ds(off, TS), :],
                                     x_v.at[pl.ds(off, TS), :],
                                     sem.at[SEM_X + c])

    def xr_copy():
        return pltpu.make_async_copy(x_hbm.at[0, pl.ds(2 * TS, S - 2 * TS), :],
                                     x_v.at[pl.ds(2 * TS, S - 2 * TS), :],
                                     sem.at[SEM_X + 2])

    def w1_copy(j):
        off = pl.multiple_of(j * TF, TF)
        return pltpu.make_async_copy(w1_hbm.at[:, pl.ds(off, TF)],
                                     w1_v.at[j], sem.at[SEM_W1 + j])

    def w2_copy(c):
        off = pl.multiple_of(c * TS, TS)
        return pltpu.make_async_copy(w2_hbm.at[:, pl.ds(off, TS)],
                                     w2_v.at[c], sem.at[SEM_W2 + c])

    def wkv_copy():
        return pltpu.make_async_copy(wqkv_hbm.at[:, pl.ds(D, 2 * D)], wkv_v,
                                     sem.at[SEM_WKV])

    def wq_copy():
        return pltpu.make_async_copy(wqkv_hbm.at[:, pl.ds(0, D)], wq_v,
                                     sem.at[SEM_WQ])

    def wo_copy():
        return pltpu.make_async_copy(wo_hbm, wo_v, sem.at[SEM_WO])

    @pl.when(step == 0)
    def _stats():
        x_copy(0).start()
        wkv_copy().start()
        x_copy(1).start()
        z_row = jnp.zeros((1, D), jnp.float32)
        for c in range(NS):
            if c == 0:
                x_copy(0).wait()
                xr_copy().start()
            elif c == 1:
                x_copy(1).wait()
                for j in range(NF):
                    w1_copy(j).start()
            elif c == 2:
                xr_copy().wait()
            xb = x_v[c * TS:(c + 1) * TS, :]
            xc = xb.astype(jnp.float32)
            m = jnp.mean(xc, axis=-1, keepdims=True)
            xm = xc - m
            var = jnp.mean(xm * xm, axis=-1, keepdims=True)
            h = xm / jnp.sqrt(var + 1e-5)
            hT_ref[:, c * TS:(c + 1) * TS] = h.T.astype(jnp.bfloat16)
            if c == 0:
                wkv_copy().wait()
            kv = jnp.dot(xb, wkv_v[...],
                         preferred_element_type=jnp.float32)
            pk = _phi(kv[:, :D])
            z_row = z_row + jnp.sum(pk, axis=0, keepdims=True)
            pkb = pk.astype(jnp.bfloat16)
            vb = kv[:, D:].astype(jnp.bfloat16)
            for g in range(NG):
                part = jax.lax.dot_general(
                    pkb[:, g * G:(g + 1) * G], vb[:, g * G:(g + 1) * G],
                    (((0,), (0,)), ((), ())),
                    preferred_element_type=jnp.float32)
                if c == 0:
                    kv_ref[g] = part
                else:
                    kv_ref[g] += part
        ri = jax.lax.broadcasted_iota(jnp.int32, (G, G), 0) // DH
        ci = jax.lax.broadcasted_iota(jnp.int32, (G, G), 1) // DH
        mask = ri == ci
        for g in range(NG):
            zb = jnp.broadcast_to(z_row[:, g * G:(g + 1) * G], (G, G)).T
            w_ref[g * G:(g + 1) * G, 0:G] = jnp.where(
                mask, kv_ref[g], 0.0).astype(jnp.bfloat16)
            w_ref[g * G:(g + 1) * G, G:2 * G] = jnp.where(
                mask, zb, 0.0).astype(jnp.bfloat16)

    @pl.when(step == 1)
    def _mixer1():
        for c in range(NS):
            w2_copy(c).start()
        wq_copy().start()
        wo_copy().start()
        for j in range(NF):
            w1_copy(j).wait()
        for j in range(NF):
            u = jnp.dot(hT_ref[...], w1_v[j],
                        preferred_element_type=jnp.float32)
            u = u + b1_ref[j * TF:(j + 1) * TF].reshape(1, TF).astype(
                jnp.float32)
            u_ref[:, j * TF:(j + 1) * TF] = jax.nn.gelu(
                u, approximate=True).astype(jnp.bfloat16)

    @pl.when(step >= 2)
    def _out():
        cs = step - 2

        @pl.when(cs == 0)
        def _():
            wq_copy().wait()
            wo_copy().wait()

        for r in range(CPS):
            w2_copy(cs * CPS + r).wait()
        for r in range(CPS):
            c = cs * CPS + r
            off = pl.multiple_of(c * TS, TS)
            xb = x_v[pl.ds(off, TS), :]
            xc = xb.astype(jnp.float32)
            y = jnp.dot(u_ref[...], w2_v[c],
                        preferred_element_type=jnp.float32)
            y = y + b2_ref[pl.ds(off, TS)].reshape(1, TS).astype(jnp.float32)
            b = y.T
            gl = jnp.sum(xc * gw_ref[...].reshape(1, D).astype(jnp.float32),
                         axis=-1, keepdims=True)
            gate = jax.nn.sigmoid(gl)
            q = jnp.dot(xb, wq_v[...], preferred_element_type=jnp.float32)
            pq = _phi(q).astype(jnp.bfloat16)
            os = []
            for g in range(NG):
                nd = jnp.dot(pq[:, g * G:(g + 1) * G],
                             w_ref[g * G:(g + 1) * G, :],
                             preferred_element_type=jnp.float32)
                os.append(nd[:, :G] / (nd[:, G:] + 1e-6))
            o = jnp.concatenate(os, axis=-1).astype(jnp.bfloat16)
            a = jnp.dot(o, wo_v[...], preferred_element_type=jnp.float32)
            o_ref[r * TS:(r + 1) * TS, :] = (
                gate * a + (1.0 - gate) * b).astype(o_ref.dtype)


@jax.jit
def pallas_gated_mix__linear_attn_block__mixer_token_mlp__prompt_kernel(
    A_x: jax.Array,
    A_wqkv: jax.Array,
    A_wo: jax.Array,
    B_x: jax.Array,
    B_w1: jax.Array,
    B_b1: jax.Array,
    B_w2: jax.Array,
    B_b2: jax.Array,
    gate_w: jax.Array,
):
    nout = 2

    out = pl.pallas_call(
        _kernel,
        grid=(2 + NS // CPS,),
        in_specs=[
            pl.BlockSpec(memory_space=pl.ANY),
            pl.BlockSpec(memory_space=pl.ANY),
            pl.BlockSpec(memory_space=pl.ANY),
            pl.BlockSpec(memory_space=pl.ANY),
            pl.BlockSpec(memory_space=pl.ANY),
            pl.BlockSpec((F,), lambda i: (0,)),
            pl.BlockSpec((S,), lambda i: (0,)),
            pl.BlockSpec((D,), lambda i: (0,)),
        ],
        out_specs=pl.BlockSpec((None, CPS * TS, D),
                               lambda i: (0, jnp.maximum(i - nout, 0), 0)),
        out_shape=jax.ShapeDtypeStruct((1, S, D), A_x.dtype),
        scratch_shapes=[
            pltpu.VMEM((S, D), jnp.bfloat16),
            pltpu.VMEM((D, 2 * D), jnp.bfloat16),
            pltpu.VMEM((D, D), jnp.bfloat16),
            pltpu.VMEM((D, D), jnp.bfloat16),
            pltpu.VMEM((NF, S, TF), jnp.bfloat16),
            pltpu.VMEM((NS, F, TS), jnp.bfloat16),
            pltpu.VMEM((D, S), jnp.bfloat16),
            pltpu.VMEM((D, F), jnp.bfloat16),
            pltpu.VMEM((NG, G, G), jnp.float32),
            pltpu.VMEM((D, 2 * G), jnp.bfloat16),
            pltpu.SemaphoreType.DMA((NSEM,)),
        ],
        compiler_params=pltpu.CompilerParams(
            dimension_semantics=("arbitrary",),
            vmem_limit_bytes=64 * 1024 * 1024,
        ),
    )(A_x, A_wqkv, A_wo, B_w1, B_w2, B_b1, B_b2, gate_w)
    return out
```

```python
import jax
import jax.numpy as jnp
import jax.experimental.pallas as pl
import jax.experimental.pallas.tpu as pltpu

S, D, F = 2048, 512, 1792
H = 32
DH = D // H
G = 128
NG = D // G
TF = 256
TS = 256
NF = F // TF
NS = S // TS
CPS = 2

SEM_X = 0
SEM_W1 = SEM_X + NS
SEM_W2 = SEM_W1 + NF
SEM_WKV = SEM_W2 + NS
SEM_WQ = SEM_WKV + 1
SEM_WO = SEM_WQ + 1
NSEM = SEM_WO + 1


def _phi(t):
    return jnp.where(t > 0, t + 1.0, jnp.exp(t)) + 1e-6


def _kernel(x_hbm, wqkv_hbm, wo_hbm, w1_hbm, w2_hbm, b1_ref, b2_ref, gw_ref,
            o_ref,
            x_v, wkv_v, wq_v, wo_v, w1_v, w2_v, hT_ref, u_ref, kv_ref,
            w_ref, sem):
    step = pl.program_id(0)

    def x_copy(c):
        off = pl.multiple_of(c * TS, TS)
        return pltpu.make_async_copy(x_hbm.at[0, pl.ds(off, TS), :],
                                     x_v.at[pl.ds(off, TS), :],
                                     sem.at[SEM_X + c])

    def xr_copy():
        return pltpu.make_async_copy(x_hbm.at[0, pl.ds(2 * TS, S - 2 * TS), :],
                                     x_v.at[pl.ds(2 * TS, S - 2 * TS), :],
                                     sem.at[SEM_X + 2])

    def w1_copy(j):
        off = pl.multiple_of(j * TF, TF)
        return pltpu.make_async_copy(w1_hbm.at[:, pl.ds(off, TF)],
                                     w1_v.at[j], sem.at[SEM_W1 + j])

    def w2_copy(c):
        off = pl.multiple_of(c * TS, TS)
        return pltpu.make_async_copy(w2_hbm.at[:, pl.ds(off, TS)],
                                     w2_v.at[c], sem.at[SEM_W2 + c])

    def wkv_copy():
        return pltpu.make_async_copy(wqkv_hbm.at[:, pl.ds(D, 2 * D)], wkv_v,
                                     sem.at[SEM_WKV])

    def wq_copy():
        return pltpu.make_async_copy(wqkv_hbm.at[:, pl.ds(0, D)], wq_v,
                                     sem.at[SEM_WQ])

    def wo_copy():
        return pltpu.make_async_copy(wo_hbm, wo_v, sem.at[SEM_WO])

    @pl.when(step == 0)
    def _stats():
        x_copy(0).start()
        wkv_copy().start()
        x_copy(1).start()
        z_row = jnp.zeros((1, D), jnp.float32)
        for c in range(NS):
            if c == 0:
                x_copy(0).wait()
                xr_copy().start()
            elif c == 1:
                x_copy(1).wait()
                for j in range(NF):
                    w1_copy(j).start()
            elif c == 2:
                xr_copy().wait()
            xb = x_v[c * TS:(c + 1) * TS, :]
            xc = xb.astype(jnp.float32)
            m = jnp.mean(xc, axis=-1, keepdims=True)
            xm = xc - m
            var = jnp.mean(xm * xm, axis=-1, keepdims=True)
            h = xm / jnp.sqrt(var + 1e-5)
            hT_ref[:, c * TS:(c + 1) * TS] = h.T.astype(jnp.bfloat16)
            if c == 0:
                wkv_copy().wait()
            kv = jnp.dot(xb, wkv_v[...],
                         preferred_element_type=jnp.float32)
            pk = _phi(kv[:, :D])
            z_row = z_row + jnp.sum(pk, axis=0, keepdims=True)
            pkT = pk.T.astype(jnp.bfloat16)
            vb = kv[:, D:].astype(jnp.bfloat16)
            for g in range(NG):
                part = jnp.dot(pkT[g * G:(g + 1) * G, :],
                               vb[:, g * G:(g + 1) * G],
                               preferred_element_type=jnp.float32)
                if c == 0:
                    kv_ref[g] = part
                else:
                    kv_ref[g] += part
        ri = jax.lax.broadcasted_iota(jnp.int32, (G, G), 0) // DH
        ci = jax.lax.broadcasted_iota(jnp.int32, (G, G), 1) // DH
        mask = ri == ci
        for g in range(NG):
            zb = jnp.broadcast_to(z_row[:, g * G:(g + 1) * G], (G, G)).T
            w_ref[g * G:(g + 1) * G, 0:G] = jnp.where(
                mask, kv_ref[g], 0.0).astype(jnp.bfloat16)
            w_ref[g * G:(g + 1) * G, G:2 * G] = jnp.where(
                mask, zb, 0.0).astype(jnp.bfloat16)

    @pl.when(step == 1)
    def _mixer1():
        for c in range(NS):
            w2_copy(c).start()
        wq_copy().start()
        wo_copy().start()
        for j in range(NF):
            w1_copy(j).wait()
        for j in range(NF):
            u = jnp.dot(hT_ref[...], w1_v[j],
                        preferred_element_type=jnp.float32)
            u = u + b1_ref[j * TF:(j + 1) * TF].reshape(1, TF).astype(
                jnp.float32)
            u_ref[:, j * TF:(j + 1) * TF] = jax.nn.gelu(
                u, approximate=True).astype(jnp.bfloat16)

    @pl.when(step >= 2)
    def _out():
        cs = step - 2

        @pl.when(cs == 0)
        def _():
            wq_copy().wait()
            wo_copy().wait()

        for r in range(CPS):
            w2_copy(cs * CPS + r).wait()
        def y_part(c, off):
            y = jnp.dot(u_ref[...], w2_v[c],
                        preferred_element_type=jnp.float32)
            y = y + b2_ref[pl.ds(off, TS)].reshape(1, TS).astype(jnp.float32)
            return y.T

        def att_part(off):
            xb = x_v[pl.ds(off, TS), :]
            xc = xb.astype(jnp.float32)
            gl = jnp.sum(xc * gw_ref[...].reshape(1, D).astype(jnp.float32),
                         axis=-1, keepdims=True)
            gate = jax.nn.sigmoid(gl)
            q = jnp.dot(xb, wq_v[...], preferred_element_type=jnp.float32)
            pq = _phi(q).astype(jnp.bfloat16)
            os = []
            for g in range(NG):
                nd = jnp.dot(pq[:, g * G:(g + 1) * G],
                             w_ref[g * G:(g + 1) * G, :],
                             preferred_element_type=jnp.float32)
                os.append(nd[:, :G] / (nd[:, G:] + 1e-6))
            o = jnp.concatenate(os, axis=-1).astype(jnp.bfloat16)
            a = jnp.dot(o, wo_v[...], preferred_element_type=jnp.float32)
            return gate, a

        cc = [cs * CPS + r for r in range(CPS)]
        offs = [pl.multiple_of(c * TS, TS) for c in cc]
        b0 = y_part(cc[0], offs[0])
        g0, a0 = att_part(offs[0])
        o_ref[0:TS, :] = (g0 * a0 + (1.0 - g0) * b0).astype(o_ref.dtype)
        g1, a1 = att_part(offs[1])
        b1 = y_part(cc[1], offs[1])
        o_ref[TS:2 * TS, :] = (g1 * a1 + (1.0 - g1) * b1).astype(o_ref.dtype)


@jax.jit
def pallas_gated_mix__linear_attn_block__mixer_token_mlp__prompt_kernel(
    A_x: jax.Array,
    A_wqkv: jax.Array,
    A_wo: jax.Array,
    B_x: jax.Array,
    B_w1: jax.Array,
    B_b1: jax.Array,
    B_w2: jax.Array,
    B_b2: jax.Array,
    gate_w: jax.Array,
):
    nout = 2

    out = pl.pallas_call(
        _kernel,
        grid=(2 + NS // CPS,),
        in_specs=[
            pl.BlockSpec(memory_space=pl.ANY),
            pl.BlockSpec(memory_space=pl.ANY),
            pl.BlockSpec(memory_space=pl.ANY),
            pl.BlockSpec(memory_space=pl.ANY),
            pl.BlockSpec(memory_space=pl.ANY),
            pl.BlockSpec((F,), lambda i: (0,)),
            pl.BlockSpec((S,), lambda i: (0,)),
            pl.BlockSpec((D,), lambda i: (0,)),
        ],
        out_specs=pl.BlockSpec((None, CPS * TS, D),
                               lambda i: (0, jnp.maximum(i - nout, 0), 0)),
        out_shape=jax.ShapeDtypeStruct((1, S, D), A_x.dtype),
        scratch_shapes=[
            pltpu.VMEM((S, D), jnp.bfloat16),
            pltpu.VMEM((D, 2 * D), jnp.bfloat16),
            pltpu.VMEM((D, D), jnp.bfloat16),
            pltpu.VMEM((D, D), jnp.bfloat16),
            pltpu.VMEM((NF, S, TF), jnp.bfloat16),
            pltpu.VMEM((NS, F, TS), jnp.bfloat16),
            pltpu.VMEM((D, S), jnp.bfloat16),
            pltpu.VMEM((D, F), jnp.bfloat16),
            pltpu.VMEM((NG, G, G), jnp.float32),
            pltpu.VMEM((D, 2 * G), jnp.bfloat16),
            pltpu.SemaphoreType.DMA((NSEM,)),
        ],
        compiler_params=pltpu.CompilerParams(
            dimension_semantics=("arbitrary",),
            vmem_limit_bytes=64 * 1024 * 1024,
        ),
    )(A_x, A_wqkv, A_wo, B_w1, B_w2, B_b1, B_b2, gate_w)
    return out
```

```python
import jax
import jax.numpy as jnp
import jax.experimental.pallas as pl
import jax.experimental.pallas.tpu as pltpu

S, D, F = 2048, 512, 1792
H = 32
DH = D // H
G = 128
NG = D // G
TF = 256
TS = 256
NF = F // TF
NS = S // TS
CPS = 2

SEM_X = 0
SEM_W1 = SEM_X + NS
SEM_W2 = SEM_W1 + NF
SEM_WKV = SEM_W2 + NS
SEM_WQ = SEM_WKV + 1
SEM_WO = SEM_WQ + 1
NSEM = SEM_WO + 1


def _phi(t):
    return jnp.where(t > 0, t + 1.0, jnp.exp(t)) + 1e-6


def _kernel(x_hbm, wqkv_hbm, wo_hbm, w1_hbm, w2_hbm, b1_ref, b2_ref, gw_ref,
            o_ref,
            x_v, wkv_v, wq_v, wo_v, w1_v, w2_v, hT_ref, u_ref, kv_ref,
            w_ref, sem):
    step = pl.program_id(0)

    def x_copy(c):
        off = pl.multiple_of(c * TS, TS)
        return pltpu.make_async_copy(x_hbm.at[0, pl.ds(off, TS), :],
                                     x_v.at[pl.ds(off, TS), :],
                                     sem.at[SEM_X + c])

    def xr_copy():
        return pltpu.make_async_copy(x_hbm.at[0, pl.ds(2 * TS, S - 2 * TS), :],
                                     x_v.at[pl.ds(2 * TS, S - 2 * TS), :],
                                     sem.at[SEM_X + 2])

    def w1_copy(j):
        off = pl.multiple_of(j * TF, TF)
        return pltpu.make_async_copy(w1_hbm.at[:, pl.ds(off, TF)],
                                     w1_v.at[j], sem.at[SEM_W1 + j])

    def w2_copy(c):
        off = pl.multiple_of(c * TS, TS)
        return pltpu.make_async_copy(w2_hbm.at[:, pl.ds(off, TS)],
                                     w2_v.at[c], sem.at[SEM_W2 + c])

    def wkv_copy():
        return pltpu.make_async_copy(wqkv_hbm.at[:, pl.ds(D, 2 * D)], wkv_v,
                                     sem.at[SEM_WKV])

    def wq_copy():
        return pltpu.make_async_copy(wqkv_hbm.at[:, pl.ds(0, D)], wq_v,
                                     sem.at[SEM_WQ])

    def wo_copy():
        return pltpu.make_async_copy(wo_hbm, wo_v, sem.at[SEM_WO])

    @pl.when(step == 0)
    def _stats():
        x_copy(0).start()
        wkv_copy().start()
        x_copy(1).start()
        z_row = jnp.zeros((1, D), jnp.float32)
        for c in range(NS):
            if c == 0:
                x_copy(0).wait()
                xr_copy().start()
            elif c == 1:
                x_copy(1).wait()
                for j in range(NF):
                    w1_copy(j).start()
            elif c == 2:
                xr_copy().wait()
            xb = x_v[c * TS:(c + 1) * TS, :]
            xc = xb.astype(jnp.float32)
            m = jnp.mean(xc, axis=-1, keepdims=True)
            xm = xc - m
            var = jnp.mean(xm * xm, axis=-1, keepdims=True)
            h = xm * jax.lax.rsqrt(var + 1e-5)
            hT_ref[:, c * TS:(c + 1) * TS] = h.T.astype(jnp.bfloat16)
            if c == 0:
                wkv_copy().wait()
            kv = jnp.dot(xb, wkv_v[...],
                         preferred_element_type=jnp.float32)
            pk = _phi(kv[:, :D])
            z_row = z_row + jnp.sum(pk, axis=0, keepdims=True)
            pkT = pk.T.astype(jnp.bfloat16)
            vb = kv[:, D:].astype(jnp.bfloat16)
            for g in range(NG):
                part = jnp.dot(pkT[g * G:(g + 1) * G, :],
                               vb[:, g * G:(g + 1) * G],
                               preferred_element_type=jnp.float32)
                if c == 0:
                    kv_ref[g] = part
                else:
                    kv_ref[g] += part
        ri = jax.lax.broadcasted_iota(jnp.int32, (G, G), 0) // DH
        ci = jax.lax.broadcasted_iota(jnp.int32, (G, G), 1) // DH
        mask = ri == ci
        for g in range(NG):
            zb = jnp.broadcast_to(z_row[:, g * G:(g + 1) * G], (G, G)).T
            w_ref[g * G:(g + 1) * G, 0:G] = jnp.where(
                mask, kv_ref[g], 0.0).astype(jnp.bfloat16)
            w_ref[g * G:(g + 1) * G, G:2 * G] = jnp.where(
                mask, zb, 0.0).astype(jnp.bfloat16)

    @pl.when(step == 1)
    def _mixer1():
        for c in range(NS):
            w2_copy(c).start()
        wq_copy().start()
        wo_copy().start()
        for j in range(NF):
            w1_copy(j).wait()
        for j in range(NF):
            u = jnp.dot(hT_ref[...], w1_v[j],
                        preferred_element_type=jnp.float32)
            u = u + b1_ref[j * TF:(j + 1) * TF].reshape(1, TF).astype(
                jnp.float32)
            u_ref[:, j * TF:(j + 1) * TF] = jax.nn.gelu(
                u, approximate=True).astype(jnp.bfloat16)

    @pl.when(step >= 2)
    def _out():
        cs = step - 2

        @pl.when(cs == 0)
        def _():
            wq_copy().wait()
            wo_copy().wait()

        for r in range(CPS):
            w2_copy(cs * CPS + r).wait()
        for r in range(CPS):
            c = cs * CPS + r
            off = pl.multiple_of(c * TS, TS)
            xb = x_v[pl.ds(off, TS), :]
            xc = xb.astype(jnp.float32)
            y = jnp.dot(u_ref[...], w2_v[c],
                        preferred_element_type=jnp.float32)
            y = y + b2_ref[pl.ds(off, TS)].reshape(1, TS).astype(jnp.float32)
            b = y.T
            gl = jnp.sum(xc * gw_ref[...].reshape(1, D).astype(jnp.float32),
                         axis=-1, keepdims=True)
            gate = jax.nn.sigmoid(gl)
            q = jnp.dot(xb, wq_v[...], preferred_element_type=jnp.float32)
            pq = _phi(q).astype(jnp.bfloat16)
            os = []
            for g in range(NG):
                nd = jnp.dot(pq[:, g * G:(g + 1) * G],
                             w_ref[g * G:(g + 1) * G, :],
                             preferred_element_type=jnp.float32)
                os.append(nd[:, :G] / (nd[:, G:] + 1e-6))
            o = jnp.concatenate(os, axis=-1).astype(jnp.bfloat16)
            a = jnp.dot(o, wo_v[...], preferred_element_type=jnp.float32)
            o_ref[r * TS:(r + 1) * TS, :] = (
                gate * a + (1.0 - gate) * b).astype(o_ref.dtype)


@jax.jit
def pallas_gated_mix__linear_attn_block__mixer_token_mlp__prompt_kernel(
    A_x: jax.Array,
    A_wqkv: jax.Array,
    A_wo: jax.Array,
    B_x: jax.Array,
    B_w1: jax.Array,
    B_b1: jax.Array,
    B_w2: jax.Array,
    B_b2: jax.Array,
    gate_w: jax.Array,
):
    nout = 2

    out = pl.pallas_call(
        _kernel,
        grid=(2 + NS // CPS,),
        in_specs=[
            pl.BlockSpec(memory_space=pl.ANY),
            pl.BlockSpec(memory_space=pl.ANY),
            pl.BlockSpec(memory_space=pl.ANY),
            pl.BlockSpec(memory_space=pl.ANY),
            pl.BlockSpec(memory_space=pl.ANY),
            pl.BlockSpec((F,), lambda i: (0,)),
            pl.BlockSpec((S,), lambda i: (0,)),
            pl.BlockSpec((D,), lambda i: (0,)),
        ],
        out_specs=pl.BlockSpec((None, CPS * TS, D),
                               lambda i: (0, jnp.maximum(i - nout, 0), 0)),
        out_shape=jax.ShapeDtypeStruct((1, S, D), A_x.dtype),
        scratch_shapes=[
            pltpu.VMEM((S, D), jnp.bfloat16),
            pltpu.VMEM((D, 2 * D), jnp.bfloat16),
            pltpu.VMEM((D, D), jnp.bfloat16),
            pltpu.VMEM((D, D), jnp.bfloat16),
            pltpu.VMEM((NF, S, TF), jnp.bfloat16),
            pltpu.VMEM((NS, F, TS), jnp.bfloat16),
            pltpu.VMEM((D, S), jnp.bfloat16),
            pltpu.VMEM((D, F), jnp.bfloat16),
            pltpu.VMEM((NG, G, G), jnp.float32),
            pltpu.VMEM((D, 2 * G), jnp.bfloat16),
            pltpu.SemaphoreType.DMA((NSEM,)),
        ],
        compiler_params=pltpu.CompilerParams(
            dimension_semantics=("arbitrary",),
            vmem_limit_bytes=64 * 1024 * 1024,
        ),
    )(A_x, A_wqkv, A_wo, B_w1, B_w2, B_b1, B_b2, gate_w)
    return out
```

```python
import jax
import jax.numpy as jnp
import jax.experimental.pallas as pl
import jax.experimental.pallas.tpu as pltpu

S, D, F = 2048, 512, 1792
H = 32
DH = D // H
G = 128
NG = D // G
TF = 256
TS = 256
NF = F // TF
NS = S // TS
TO = 512
NO = S // TO

SEM_X = 0
SEM_W1 = SEM_X + NS
SEM_W2 = SEM_W1 + NF
SEM_WKV = SEM_W2 + NO
SEM_WQ = SEM_WKV + 1
SEM_WO = SEM_WQ + 1
NSEM = SEM_WO + 1


def _phi(t):
    return jnp.where(t > 0, t + 1.0, jnp.exp(t)) + 1e-6


def _kernel(x_hbm, wqkv_hbm, wo_hbm, w1_hbm, w2_hbm, b1_ref, b2_ref, gw_ref,
            o_ref,
            x_v, wkv_v, wq_v, wo_v, w1_v, w2_v, hT_ref, u_ref, kv_ref,
            w_ref, sem):
    step = pl.program_id(0)

    def x_copy(c):
        off = pl.multiple_of(c * TS, TS)
        return pltpu.make_async_copy(x_hbm.at[0, pl.ds(off, TS), :],
                                     x_v.at[pl.ds(off, TS), :],
                                     sem.at[SEM_X + c])

    def xr_copy():
        return pltpu.make_async_copy(x_hbm.at[0, pl.ds(2 * TS, S - 2 * TS), :],
                                     x_v.at[pl.ds(2 * TS, S - 2 * TS), :],
                                     sem.at[SEM_X + 2])

    def w1_copy(j):
        off = pl.multiple_of(j * TF, TF)
        return pltpu.make_async_copy(w1_hbm.at[:, pl.ds(off, TF)],
                                     w1_v.at[j], sem.at[SEM_W1 + j])

    def w2_copy(c):
        off = pl.multiple_of(c * TO, TO)
        return pltpu.make_async_copy(w2_hbm.at[:, pl.ds(off, TO)],
                                     w2_v.at[c], sem.at[SEM_W2 + c])

    def wkv_copy():
        return pltpu.make_async_copy(wqkv_hbm.at[:, pl.ds(D, 2 * D)], wkv_v,
                                     sem.at[SEM_WKV])

    def wq_copy():
        return pltpu.make_async_copy(wqkv_hbm.at[:, pl.ds(0, D)], wq_v,
                                     sem.at[SEM_WQ])

    def wo_copy():
        return pltpu.make_async_copy(wo_hbm, wo_v, sem.at[SEM_WO])

    @pl.when(step == 0)
    def _stats():
        x_copy(0).start()
        wkv_copy().start()
        x_copy(1).start()
        z_row = jnp.zeros((1, D), jnp.float32)
        for c in range(NS):
            if c == 0:
                x_copy(0).wait()
                xr_copy().start()
            elif c == 1:
                x_copy(1).wait()
                for j in range(NF):
                    w1_copy(j).start()
            elif c == 2:
                xr_copy().wait()
            xb = x_v[c * TS:(c + 1) * TS, :]
            xc = xb.astype(jnp.float32)
            m = jnp.mean(xc, axis=-1, keepdims=True)
            xm = xc - m
            var = jnp.mean(xm * xm, axis=-1, keepdims=True)
            h = xm * jax.lax.rsqrt(var + 1e-5)
            hT_ref[:, c * TS:(c + 1) * TS] = h.T.astype(jnp.bfloat16)
            if c == 0:
                wkv_copy().wait()
            kv = jnp.dot(xb, wkv_v[...],
                         preferred_element_type=jnp.float32)
            pk = _phi(kv[:, :D])
            z_row = z_row + jnp.sum(pk, axis=0, keepdims=True)
            pkT = pk.T.astype(jnp.bfloat16)
            vb = kv[:, D:].astype(jnp.bfloat16)
            for g in range(NG):
                part = jnp.dot(pkT[g * G:(g + 1) * G, :],
                               vb[:, g * G:(g + 1) * G],
                               preferred_element_type=jnp.float32)
                if c == 0:
                    kv_ref[g] = part
                else:
                    kv_ref[g] += part
        ri = jax.lax.broadcasted_iota(jnp.int32, (G, G), 0) // DH
        ci = jax.lax.broadcasted_iota(jnp.int32, (G, G), 1) // DH
        mask = ri == ci
        for g in range(NG):
            zb = jnp.broadcast_to(z_row[:, g * G:(g + 1) * G], (G, G)).T
            w_ref[g * G:(g + 1) * G, 0:G] = jnp.where(
                mask, kv_ref[g], 0.0).astype(jnp.bfloat16)
            w_ref[g * G:(g + 1) * G, G:2 * G] = jnp.where(
                mask, zb, 0.0).astype(jnp.bfloat16)

    @pl.when(step == 1)
    def _mixer1():
        for c in range(NO):
            w2_copy(c).start()
        wq_copy().start()
        wo_copy().start()
        for j in range(NF):
            w1_copy(j).wait()
        for j in range(NF):
            u = jnp.dot(hT_ref[...], w1_v[j],
                        preferred_element_type=jnp.float32)
            u = u + b1_ref[j * TF:(j + 1) * TF].reshape(1, TF).astype(
                jnp.float32)
            u_ref[:, j * TF:(j + 1) * TF] = jax.nn.gelu(
                u, approximate=True).astype(jnp.bfloat16)

    @pl.when(step >= 2)
    def _out():
        cs = step - 2

        @pl.when(cs == 0)
        def _():
            wq_copy().wait()
            wo_copy().wait()

        w2_copy(cs).wait()
        off = pl.multiple_of(cs * TO, TO)
        xb = x_v[pl.ds(off, TO), :]
        xc = xb.astype(jnp.float32)
        y = jnp.dot(u_ref[...], w2_v[cs],
                    preferred_element_type=jnp.float32)
        y = y + b2_ref[pl.ds(off, TO)].reshape(1, TO).astype(jnp.float32)
        b = y.T
        gl = jnp.sum(xc * gw_ref[...].reshape(1, D).astype(jnp.float32),
                     axis=-1, keepdims=True)
        gate = jax.nn.sigmoid(gl)
        q = jnp.dot(xb, wq_v[...], preferred_element_type=jnp.float32)
        pq = _phi(q).astype(jnp.bfloat16)
        os = []
        for g in range(NG):
            nd = jnp.dot(pq[:, g * G:(g + 1) * G],
                         w_ref[g * G:(g + 1) * G, :],
                         preferred_element_type=jnp.float32)
            os.append(nd[:, :G] / (nd[:, G:] + 1e-6))
        o = jnp.concatenate(os, axis=-1).astype(jnp.bfloat16)
        a = jnp.dot(o, wo_v[...], preferred_element_type=jnp.float32)
        o_ref[...] = (gate * a + (1.0 - gate) * b).astype(o_ref.dtype)


@jax.jit
def pallas_gated_mix__linear_attn_block__mixer_token_mlp__prompt_kernel(
    A_x: jax.Array,
    A_wqkv: jax.Array,
    A_wo: jax.Array,
    B_x: jax.Array,
    B_w1: jax.Array,
    B_b1: jax.Array,
    B_w2: jax.Array,
    B_b2: jax.Array,
    gate_w: jax.Array,
):
    nout = 2

    out = pl.pallas_call(
        _kernel,
        grid=(2 + NO,),
        in_specs=[
            pl.BlockSpec(memory_space=pl.ANY),
            pl.BlockSpec(memory_space=pl.ANY),
            pl.BlockSpec(memory_space=pl.ANY),
            pl.BlockSpec(memory_space=pl.ANY),
            pl.BlockSpec(memory_space=pl.ANY),
            pl.BlockSpec((F,), lambda i: (0,)),
            pl.BlockSpec((S,), lambda i: (0,)),
            pl.BlockSpec((D,), lambda i: (0,)),
        ],
        out_specs=pl.BlockSpec((None, TO, D),
                               lambda i: (0, jnp.maximum(i - nout, 0), 0)),
        out_shape=jax.ShapeDtypeStruct((1, S, D), A_x.dtype),
        scratch_shapes=[
            pltpu.VMEM((S, D), jnp.bfloat16),
            pltpu.VMEM((D, 2 * D), jnp.bfloat16),
            pltpu.VMEM((D, D), jnp.bfloat16),
            pltpu.VMEM((D, D), jnp.bfloat16),
            pltpu.VMEM((NF, S, TF), jnp.bfloat16),
            pltpu.VMEM((NO, F, TO), jnp.bfloat16),
            pltpu.VMEM((D, S), jnp.bfloat16),
            pltpu.VMEM((D, F), jnp.bfloat16),
            pltpu.VMEM((NG, G, G), jnp.float32),
            pltpu.VMEM((D, 2 * G), jnp.bfloat16),
            pltpu.SemaphoreType.DMA((NSEM,)),
        ],
        compiler_params=pltpu.CompilerParams(
            dimension_semantics=("arbitrary",),
            vmem_limit_bytes=64 * 1024 * 1024,
        ),
    )(A_x, A_wqkv, A_wo, B_w1, B_w2, B_b1, B_b2, gate_w)
    return out
```

```python
import jax
import jax.numpy as jnp
import jax.experimental.pallas as pl
import jax.experimental.pallas.tpu as pltpu

S, D, F = 2048, 512, 1792
H = 32
DH = D // H
G = 128
NG = D // G
TF = 256
TS = 256
NF = F // TF
NS = S // TS
STAT_CHUNKS = ((0, 256), (256, 256), (512, 512), (1024, 512), (1536, 512))
TO = 512
NO = S // TO

SEM_X = 0
SEM_W1 = SEM_X + NS
SEM_W2 = SEM_W1 + NF
SEM_WKV = SEM_W2 + NO
SEM_WQ = SEM_WKV + 1
SEM_WO = SEM_WQ + 1
NSEM = SEM_WO + 1


def _phi(t):
    return jnp.where(t > 0, t + 1.0, jnp.exp(t)) + 1e-6


def _kernel(x_hbm, wqkv_hbm, wo_hbm, w1_hbm, w2_hbm, b1_ref, b2_ref, gw_ref,
            o_ref,
            x_v, wkv_v, wq_v, wo_v, w1_v, w2_v, hT_ref, u_ref, kv_ref,
            w_ref, sem):
    step = pl.program_id(0)

    def x_copy(c):
        off = pl.multiple_of(c * TS, TS)
        return pltpu.make_async_copy(x_hbm.at[0, pl.ds(off, TS), :],
                                     x_v.at[pl.ds(off, TS), :],
                                     sem.at[SEM_X + c])

    def xr_copy():
        return pltpu.make_async_copy(x_hbm.at[0, pl.ds(2 * TS, S - 2 * TS), :],
                                     x_v.at[pl.ds(2 * TS, S - 2 * TS), :],
                                     sem.at[SEM_X + 2])

    def w1_copy(j):
        off = pl.multiple_of(j * TF, TF)
        return pltpu.make_async_copy(w1_hbm.at[:, pl.ds(off, TF)],
                                     w1_v.at[j], sem.at[SEM_W1 + j])

    def w2_copy(c):
        off = pl.multiple_of(c * TO, TO)
        return pltpu.make_async_copy(w2_hbm.at[:, pl.ds(off, TO)],
                                     w2_v.at[c], sem.at[SEM_W2 + c])

    def wkv_copy():
        return pltpu.make_async_copy(wqkv_hbm.at[:, pl.ds(D, 2 * D)], wkv_v,
                                     sem.at[SEM_WKV])

    def wq_copy():
        return pltpu.make_async_copy(wqkv_hbm.at[:, pl.ds(0, D)], wq_v,
                                     sem.at[SEM_WQ])

    def wo_copy():
        return pltpu.make_async_copy(wo_hbm, wo_v, sem.at[SEM_WO])

    @pl.when(step == 0)
    def _stats():
        x_copy(0).start()
        wkv_copy().start()
        x_copy(1).start()
        z_row = jnp.zeros((1, D), jnp.float32)
        for c, (r0, rn) in enumerate(STAT_CHUNKS):
            if c == 0:
                x_copy(0).wait()
                xr_copy().start()
            elif c == 1:
                x_copy(1).wait()
                for j in range(NF):
                    w1_copy(j).start()
            elif c == 2:
                xr_copy().wait()
            xb = x_v[r0:r0 + rn, :]
            xc = xb.astype(jnp.float32)
            m = jnp.mean(xc, axis=-1, keepdims=True)
            xm = xc - m
            var = jnp.mean(xm * xm, axis=-1, keepdims=True)
            h = xm * jax.lax.rsqrt(var + 1e-5)
            hT_ref[:, r0:r0 + rn] = h.T.astype(jnp.bfloat16)
            if c == 0:
                wkv_copy().wait()
            kv = jnp.dot(xb, wkv_v[...],
                         preferred_element_type=jnp.float32)
            pk = _phi(kv[:, :D])
            z_row = z_row + jnp.sum(pk, axis=0, keepdims=True)
            pkT = pk.T.astype(jnp.bfloat16)
            vb = kv[:, D:].astype(jnp.bfloat16)
            for g in range(NG):
                part = jnp.dot(pkT[g * G:(g + 1) * G, :],
                               vb[:, g * G:(g + 1) * G],
                               preferred_element_type=jnp.float32)
                if c == 0:
                    kv_ref[g] = part
                else:
                    kv_ref[g] += part
        ri = jax.lax.broadcasted_iota(jnp.int32, (G, G), 0) // DH
        ci = jax.lax.broadcasted_iota(jnp.int32, (G, G), 1) // DH
        mask = ri == ci
        for g in range(NG):
            zb = jnp.broadcast_to(z_row[:, g * G:(g + 1) * G], (G, G)).T
            w_ref[g * G:(g + 1) * G, 0:G] = jnp.where(
                mask, kv_ref[g], 0.0).astype(jnp.bfloat16)
            w_ref[g * G:(g + 1) * G, G:2 * G] = jnp.where(
                mask, zb, 0.0).astype(jnp.bfloat16)

    @pl.when(step == 1)
    def _mixer1():
        for c in range(NO):
            w2_copy(c).start()
        wq_copy().start()
        wo_copy().start()
        for j in range(NF):
            w1_copy(j).wait()
        for j in range(NF):
            u = jnp.dot(hT_ref[...], w1_v[j],
                        preferred_element_type=jnp.float32)
            u = u + b1_ref[j * TF:(j + 1) * TF].reshape(1, TF).astype(
                jnp.float32)
            u_ref[:, j * TF:(j + 1) * TF] = jax.nn.gelu(
                u, approximate=True).astype(jnp.bfloat16)

    @pl.when(step >= 2)
    def _out():
        cs = step - 2

        @pl.when(cs == 0)
        def _():
            wq_copy().wait()
            wo_copy().wait()

        w2_copy(cs).wait()
        off = pl.multiple_of(cs * TO, TO)
        xb = x_v[pl.ds(off, TO), :]
        xc = xb.astype(jnp.float32)
        y = jnp.dot(u_ref[...], w2_v[cs],
                    preferred_element_type=jnp.float32)
        y = y + b2_ref[pl.ds(off, TO)].reshape(1, TO).astype(jnp.float32)
        b = y.T
        gl = jnp.sum(xc * gw_ref[...].reshape(1, D).astype(jnp.float32),
                     axis=-1, keepdims=True)
        gate = jax.nn.sigmoid(gl)
        q = jnp.dot(xb, wq_v[...], preferred_element_type=jnp.float32)
        pq = _phi(q).astype(jnp.bfloat16)
        os = []
        for g in range(NG):
            nd = jnp.dot(pq[:, g * G:(g + 1) * G],
                         w_ref[g * G:(g + 1) * G, :],
                         preferred_element_type=jnp.float32)
            os.append(nd[:, :G] / (nd[:, G:] + 1e-6))
        o = jnp.concatenate(os, axis=-1).astype(jnp.bfloat16)
        a = jnp.dot(o, wo_v[...], preferred_element_type=jnp.float32)
        o_ref[...] = (gate * a + (1.0 - gate) * b).astype(o_ref.dtype)


@jax.jit
def pallas_gated_mix__linear_attn_block__mixer_token_mlp__prompt_kernel(
    A_x: jax.Array,
    A_wqkv: jax.Array,
    A_wo: jax.Array,
    B_x: jax.Array,
    B_w1: jax.Array,
    B_b1: jax.Array,
    B_w2: jax.Array,
    B_b2: jax.Array,
    gate_w: jax.Array,
):
    nout = 2

    out = pl.pallas_call(
        _kernel,
        grid=(2 + NO,),
        in_specs=[
            pl.BlockSpec(memory_space=pl.ANY),
            pl.BlockSpec(memory_space=pl.ANY),
            pl.BlockSpec(memory_space=pl.ANY),
            pl.BlockSpec(memory_space=pl.ANY),
            pl.BlockSpec(memory_space=pl.ANY),
            pl.BlockSpec((F,), lambda i: (0,)),
            pl.BlockSpec((S,), lambda i: (0,)),
            pl.BlockSpec((D,), lambda i: (0,)),
        ],
        out_specs=pl.BlockSpec((None, TO, D),
                               lambda i: (0, jnp.maximum(i - nout, 0), 0)),
        out_shape=jax.ShapeDtypeStruct((1, S, D), A_x.dtype),
        scratch_shapes=[
            pltpu.VMEM((S, D), jnp.bfloat16),
            pltpu.VMEM((D, 2 * D), jnp.bfloat16),
            pltpu.VMEM((D, D), jnp.bfloat16),
            pltpu.VMEM((D, D), jnp.bfloat16),
            pltpu.VMEM((NF, S, TF), jnp.bfloat16),
            pltpu.VMEM((NO, F, TO), jnp.bfloat16),
            pltpu.VMEM((D, S), jnp.bfloat16),
            pltpu.VMEM((D, F), jnp.bfloat16),
            pltpu.VMEM((NG, G, G), jnp.float32),
            pltpu.VMEM((D, 2 * G), jnp.bfloat16),
            pltpu.SemaphoreType.DMA((NSEM,)),
        ],
        compiler_params=pltpu.CompilerParams(
            dimension_semantics=("arbitrary",),
            vmem_limit_bytes=64 * 1024 * 1024,
        ),
    )(A_x, A_wqkv, A_wo, B_w1, B_w2, B_b1, B_b2, gate_w)
    return out
```

```python
import jax
import jax.numpy as jnp
import jax.experimental.pallas as pl
import jax.experimental.pallas.tpu as pltpu

S, D, F = 2048, 512, 1792
H = 32
DH = D // H
G = 128
NG = D // G
TF = 256
TS = 256
NF = F // TF
NS = S // TS
TO = 512
NO = S // TO

SEM_X = 0
SEM_W1 = SEM_X + NS
SEM_W2 = SEM_W1 + NF
SEM_WKV = SEM_W2 + NO
SEM_WQ = SEM_WKV + 1
SEM_WO = SEM_WQ + 1
NSEM = SEM_WO + 1


def _phi(t):
    return jnp.where(t > 0, t + 1.0, jnp.exp(t)) + 1e-6


def _kernel(x_hbm, wqkv_hbm, wo_hbm, w1_hbm, w2_hbm, b1_ref, b2_ref, gw_ref,
            o_ref,
            x_v, wkv_v, wq_v, wo_v, w1_v, w2_v, hT_ref, u_ref, kv_ref, z_ref,
            w_ref, sem):
    step = pl.program_id(0)

    def x_copy(c):
        off = pl.multiple_of(c * TS, TS)
        return pltpu.make_async_copy(x_hbm.at[0, pl.ds(off, TS), :],
                                     x_v.at[pl.ds(off, TS), :],
                                     sem.at[SEM_X + c])

    def xr_copy():
        return pltpu.make_async_copy(x_hbm.at[0, pl.ds(2 * TS, S - 2 * TS), :],
                                     x_v.at[pl.ds(2 * TS, S - 2 * TS), :],
                                     sem.at[SEM_X + 2])

    def w1_copy(j):
        off = pl.multiple_of(j * TF, TF)
        return pltpu.make_async_copy(w1_hbm.at[:, pl.ds(off, TF)],
                                     w1_v.at[j], sem.at[SEM_W1 + j])

    def w2_copy(c):
        off = pl.multiple_of(c * TO, TO)
        return pltpu.make_async_copy(w2_hbm.at[:, pl.ds(off, TO)],
                                     w2_v.at[c], sem.at[SEM_W2 + c])

    def wkv_copy():
        return pltpu.make_async_copy(wqkv_hbm.at[:, pl.ds(D, 2 * D)], wkv_v,
                                     sem.at[SEM_WKV])

    def wq_copy():
        return pltpu.make_async_copy(wqkv_hbm.at[:, pl.ds(0, D)], wq_v,
                                     sem.at[SEM_WQ])

    def wo_copy():
        return pltpu.make_async_copy(wo_hbm, wo_v, sem.at[SEM_WO])

    @pl.when(step == 0)
    def _stats():
        x_copy(0).start()
        wkv_copy().start()
        x_copy(1).start()
        z_row = jnp.zeros((1, D), jnp.float32)
        for c in range(NS):
            if c == 0:
                x_copy(0).wait()
                xr_copy().start()
            elif c == 1:
                x_copy(1).wait()
                for j in range(NF):
                    w1_copy(j).start()
            elif c == 2:
                xr_copy().wait()
            xb = x_v[c * TS:(c + 1) * TS, :]
            xc = xb.astype(jnp.float32)
            m = jnp.mean(xc, axis=-1, keepdims=True)
            xm = xc - m
            var = jnp.mean(xm * xm, axis=-1, keepdims=True)
            h = xm * jax.lax.rsqrt(var + 1e-5)
            hT_ref[:, c * TS:(c + 1) * TS] = h.T.astype(jnp.bfloat16)
            if c == 0:
                wkv_copy().wait()
            kv = jnp.dot(xb, wkv_v[...],
                         preferred_element_type=jnp.float32)
            pk = _phi(kv[:, :D])
            z_row = z_row + jnp.sum(pk, axis=0, keepdims=True)
            pkT = pk.T.astype(jnp.bfloat16)
            vb = kv[:, D:].astype(jnp.bfloat16)
            for g in range(NG):
                part = jnp.dot(pkT[g * G:(g + 1) * G, :],
                               vb[:, g * G:(g + 1) * G],
                               preferred_element_type=jnp.float32)
                if c == 0:
                    kv_ref[g] = part
                else:
                    kv_ref[g] += part
        z_ref[...] = z_row

    @pl.when(step == 1)
    def _mixer1():
        for c in range(NO):
            w2_copy(c).start()
        wq_copy().start()
        wo_copy().start()
        for j in range(NF):
            w1_copy(j).wait()
        ri = jax.lax.broadcasted_iota(jnp.int32, (G, G), 0) // DH
        ci = jax.lax.broadcasted_iota(jnp.int32, (G, G), 1) // DH
        mask = ri == ci
        for g in range(NG):
            zb = jnp.broadcast_to(z_ref[:, g * G:(g + 1) * G], (G, G)).T
            w_ref[g * G:(g + 1) * G, 0:G] = jnp.where(
                mask, kv_ref[g], 0.0).astype(jnp.bfloat16)
            w_ref[g * G:(g + 1) * G, G:2 * G] = jnp.where(
                mask, zb, 0.0).astype(jnp.bfloat16)
        for j in range(NF):
            u = jnp.dot(hT_ref[...], w1_v[j],
                        preferred_element_type=jnp.float32)
            u = u + b1_ref[j * TF:(j + 1) * TF].reshape(1, TF).astype(
                jnp.float32)
            u_ref[:, j * TF:(j + 1) * TF] = jax.nn.gelu(
                u, approximate=True).astype(jnp.bfloat16)

    @pl.when(step >= 2)
    def _out():
        cs = step - 2

        @pl.when(cs == 0)
        def _():
            wq_copy().wait()
            wo_copy().wait()

        w2_copy(cs).wait()
        off = pl.multiple_of(cs * TO, TO)
        xb = x_v[pl.ds(off, TO), :]
        xc = xb.astype(jnp.float32)
        y = jnp.dot(u_ref[...], w2_v[cs],
                    preferred_element_type=jnp.float32)
        y = y + b2_ref[pl.ds(off, TO)].reshape(1, TO).astype(jnp.float32)
        b = y.T
        gl = jnp.sum(xc * gw_ref[...].reshape(1, D).astype(jnp.float32),
                     axis=-1, keepdims=True)
        gate = jax.nn.sigmoid(gl)
        q = jnp.dot(xb, wq_v[...], preferred_element_type=jnp.float32)
        pq = _phi(q).astype(jnp.bfloat16)
        os = []
        for g in range(NG):
            nd = jnp.dot(pq[:, g * G:(g + 1) * G],
                         w_ref[g * G:(g + 1) * G, :],
                         preferred_element_type=jnp.float32)
            os.append(nd[:, :G] / (nd[:, G:] + 1e-6))
        o = jnp.concatenate(os, axis=-1).astype(jnp.bfloat16)
        a = jnp.dot(o, wo_v[...], preferred_element_type=jnp.float32)
        o_ref[...] = (gate * a + (1.0 - gate) * b).astype(o_ref.dtype)


@jax.jit
def pallas_gated_mix__linear_attn_block__mixer_token_mlp__prompt_kernel(
    A_x: jax.Array,
    A_wqkv: jax.Array,
    A_wo: jax.Array,
    B_x: jax.Array,
    B_w1: jax.Array,
    B_b1: jax.Array,
    B_w2: jax.Array,
    B_b2: jax.Array,
    gate_w: jax.Array,
):
    nout = 2

    out = pl.pallas_call(
        _kernel,
        grid=(2 + NO,),
        in_specs=[
            pl.BlockSpec(memory_space=pl.ANY),
            pl.BlockSpec(memory_space=pl.ANY),
            pl.BlockSpec(memory_space=pl.ANY),
            pl.BlockSpec(memory_space=pl.ANY),
            pl.BlockSpec(memory_space=pl.ANY),
            pl.BlockSpec((F,), lambda i: (0,)),
            pl.BlockSpec((S,), lambda i: (0,)),
            pl.BlockSpec((D,), lambda i: (0,)),
        ],
        out_specs=pl.BlockSpec((None, TO, D),
                               lambda i: (0, jnp.maximum(i - nout, 0), 0)),
        out_shape=jax.ShapeDtypeStruct((1, S, D), A_x.dtype),
        scratch_shapes=[
            pltpu.VMEM((S, D), jnp.bfloat16),
            pltpu.VMEM((D, 2 * D), jnp.bfloat16),
            pltpu.VMEM((D, D), jnp.bfloat16),
            pltpu.VMEM((D, D), jnp.bfloat16),
            pltpu.VMEM((NF, S, TF), jnp.bfloat16),
            pltpu.VMEM((NO, F, TO), jnp.bfloat16),
            pltpu.VMEM((D, S), jnp.bfloat16),
            pltpu.VMEM((D, F), jnp.bfloat16),
            pltpu.VMEM((NG, G, G), jnp.float32),
            pltpu.VMEM((1, D), jnp.float32),
            pltpu.VMEM((D, 2 * G), jnp.bfloat16),
            pltpu.SemaphoreType.DMA((NSEM,)),
        ],
        compiler_params=pltpu.CompilerParams(
            dimension_semantics=("arbitrary",),
            vmem_limit_bytes=64 * 1024 * 1024,
        ),
    )(A_x, A_wqkv, A_wo, B_w1, B_w2, B_b1, B_b2, gate_w)
    return out
```
